```python
import os as _os
_os.environ.setdefault("JAX_PLATFORMS", "cpu")
import jax
import jax.numpy as jnp

def _softmax(x, axis=-1):
    return jax.nn.softmax(x, axis=axis)
def _gelu(x):
    return jax.nn.gelu(x, approximate=True)
def _silu(x):
    return jax.nn.silu(x)
def _sigmoid(x):
    return jax.nn.sigmoid(x)
def _layernorm(x, axis=-1, eps=1e-5):
    m = jnp.mean(x, axis=axis, keepdims=True)
    v = jnp.var(x, axis=axis, keepdims=True)
    return (x - m) / jnp.sqrt(v + eps)
def _scatter_add(tgt, idx, src, axis=0):
    return tgt.at[idx].add(src)
def _segment_sum(src, seg, n):
    return jax.ops.segment_sum(src, seg, n)
class _Rng:
    def __init__(self, key):
        self._k = key
    def _next(self):
        self._k, sub = jax.random.split(self._k)
        return sub
    def normal(self, shape):
        return jax.random.normal(self._next(), shape, dtype=jnp.bfloat16)
    def randint(self, lo, hi, shape):
        return jax.random.randint(self._next(), shape, lo, hi, dtype=jnp.int32)
    def uniform(self, shape, lo=0.0, hi=1.0):
        return jax.random.uniform(self._next(), shape, jnp.bfloat16, lo, hi)
    def permutation(self, n):
        return jax.random.permutation(self._next(), n)


kernel_name = 'sequential_preLN__softmax_full_mha__dense_activation_gelu__prompt'

def setup_inputs():
    _rng = _Rng(jax.random.key(int.from_bytes(__import__("os").urandom(4), "little")))
    _w = (lambda a: (lambda t: t.astype(jnp.bfloat16) if jnp.issubdtype(t.dtype, jnp.floating) else t)(jnp.asarray(a)))
    def _A_setup():
        B, S, D = 1, 2048, 640
        return {
            "x": _w((lambda *s: _rng.normal(s) * 0.05)(B, S, D)),
            "wqkv": _w((lambda *s: _rng.normal(s) * 0.05)(D, 3 * D)),
            "wo": _w((lambda *s: _rng.normal(s) * 0.05)(D, D)),
        }
    _A_in = _A_setup()

    def _B_setup():
        B, S, D, F = 1, 2048, 640, 1536
        return {
            "x": _w((lambda *s: _rng.normal(s) * 0.05)(B, S, D)),
            "w1": _w((lambda *s: _rng.normal(s) * 0.4)(D, F) * (D ** -0.5)),
            "b1": _w((lambda *s: _rng.normal(s) * 0.4)(F) * 0.01),
            "w2": _w((lambda *s: _rng.normal(s) * 0.4)(F, D) * (F ** -0.5)),
            "b2": _w((lambda *s: _rng.normal(s) * 0.05)(D) * 0.01),
        }
    _B_in = _B_setup()

    return {
        "A_x": _A_in["x"],
        "A_wqkv": _A_in["wqkv"],
        "A_wo": _A_in["wo"],
        "B_x": _B_in["x"],
        "B_w1": _B_in["w1"],
        "B_b1": _B_in["b1"],
        "B_w2": _B_in["w2"],
        "B_b2": _B_in["b2"],
    }

def reference(A_x, A_wqkv, A_wo, B_x, B_w1, B_b1, B_w2, B_b2):
    def _A_ref(x, wqkv, wo):
        B, S, D = x.shape
        H = 32; Dh = D // H
        qkv = (lambda x, *d: x.transpose(*d))((x @ wqkv).reshape(B, S, 3, H, Dh), 2, 0, 3, 1, 4)
        q, k, v = qkv[0], qkv[1], qkv[2]
        scale = Dh ** -0.5
        scores = jnp.einsum("bhqd,bhkd->bhqk", q, k) * scale
        p = _softmax(scores, axis=-1)
        o = jnp.einsum("bhqk,bhkd->bhqd", p, v)
        return (lambda x, *d: x.transpose(*d))(o, 0, 2, 1, 3).reshape(B, S, D) @ wo

    def _B_ref(x, w1, b1, w2, b2):
        h = jnp.einsum("bsd,df->bsf", x, w1) + b1
        h = _gelu(h)
        return jnp.einsum("bsf,fd->bsd", h, w2) + b2

    x = A_x
    h = x + _A_ref(_layernorm(x, axis=-1), A_wqkv, A_wo)
    h2 = h + _B_ref(_layernorm(h, axis=-1), B_w1, B_b1, B_w2, B_b2)
    return h2
```

```python
import functools
import math

import jax
import jax.numpy as jnp
import jax.experimental.pallas as pl
import jax.experimental.pallas.tpu as pltpu

S = 2048
D = 640
F = 1536
H = 32
DH = D // H
NG = D // 128
EPS = 1e-5

TQ = 512
R = 128
NQ = S // TQ
NP = S // R
NT = NQ * NP
SKEW = 2
LAG = NP + SKEW
W = 24

RB = 256
NB = S // RB

QSCALE = (DH ** -0.5) * math.log2(math.e)

_NT_DIMS = (((1,), (1,)), ((), ()))


def _layernorm(x):
    m = jnp.mean(x, axis=-1, keepdims=True)
    xc = x - m
    v = jnp.mean(xc * xc, axis=-1, keepdims=True)
    return xc * jax.lax.rsqrt(v + EPS)


def _gelu(x):
    c = math.sqrt(2.0 / math.pi)
    return 0.5 * x * (1.0 + jnp.tanh(c * (x + 0.044715 * (x * x * x))))


def _kernel(x_hbm, wqkv_hbm, wo_hbm, w1_hbm, b1_hbm, w2_hbm, b2_hbm, out_hbm,
            x_v, wqkv_v, wo_v, w1_v, b1_v, w2_v, b2_v, wvt_v,
            k_ref, q_ref, vt_ref, ot_ref, m_ref, out_v, z_ref,
            sem_x, sem_w, sem_o, s0, s1, s2, s3):
    s_refs = (s0, s1, s2, s3)
    f32 = jnp.float32
    bf16 = jnp.bfloat16

    def x_copy(i):
        return pltpu.make_async_copy(
            x_hbm.at[pl.ds(i * RB, RB), :], x_v.at[pl.ds(i * RB, RB), :], sem_x.at[i])

    w_copies = [
        pltpu.make_async_copy(wqkv_hbm, wqkv_v, sem_w.at[0]),
        pltpu.make_async_copy(wo_hbm, wo_v, sem_w.at[1]),
        pltpu.make_async_copy(w1_hbm, w1_v, sem_w.at[2]),
        pltpu.make_async_copy(w2_hbm, w2_v, sem_w.at[3]),
        pltpu.make_async_copy(b1_hbm, b1_v, sem_w.at[4]),
        pltpu.make_async_copy(b2_hbm, b2_v, sem_w.at[5]),
    ]
    x_copy(0).start()
    w_copies[0].start()
    for i in range(1, NB):
        x_copy(i).start()
    for c in w_copies[1:]:
        c.start()

    z_ref[0] = 0
    z_ref[1] = 0

    w_copies[0].wait()
    wvt_v[...] = wqkv_v[:, 2 * D:3 * D].astype(f32).T.astype(bf16)

    lane_rb = jax.lax.broadcasted_iota(jnp.int32, (RB, 128), 1)

    def store_groups(ref, a, r0):
        gs = [a[:, g * 128:(g + 1) * 128] for g in range(NG)]
        gs += [jnp.where(lane_rb >= 64, gs[g], gs[g + 1]) for g in range(NG - 1)]
        for g, v in enumerate(gs):
            ref[g, pl.ds(r0, RB // 2), :] = pltpu.bitcast(v.astype(bf16), jnp.uint32)

    for i in range(NB):
        x_copy(i).wait()

    def phase_a(i, carry):
        r0 = pl.multiple_of(i * RB, RB)
        r0h = pl.multiple_of(i * (RB // 2), RB // 2)
        xn = _layernorm(x_v[pl.ds(r0, RB), :].astype(f32)).astype(bf16)
        q = jnp.dot(xn, wqkv_v[:, 0:D], preferred_element_type=f32) * QSCALE
        store_groups(q_ref, q, r0h)
        k = jnp.dot(xn, wqkv_v[:, D:2 * D], preferred_element_type=f32)
        store_groups(k_ref, k, r0h)
        vt = jax.lax.dot_general(wvt_v[...], xn, _NT_DIMS, preferred_element_type=f32)
        vt_ref[:, pl.ds(r0, RB)] = vt
        return carry

    jax.lax.fori_loop(0, NB, phase_a, 0)

    lane = jax.lax.broadcasted_iota(jnp.int32, (TQ, 128), 1)
    row = jax.lax.broadcasted_iota(jnp.int32, (W, 128), 0)

    def get_qm(h, qc):
        lo = (h * DH) & 127
        gb = (h * DH) >> 7
        g = jnp.where(lo > 128 - DH, gb + NG, gb)
        q = pltpu.bitcast(q_ref[g, qc * TQ // 2:(qc + 1) * TQ // 2, :], bf16)
        return g, jnp.where(((lane - lo) & 127) < DH, q, jnp.zeros_like(q))

    def stage_qk(z_st, g, qm, c, j, m8):
        k = pltpu.bitcast(k_ref[g, j * R // 2:(j + 1) * R // 2, :], bf16)
        s = jax.lax.dot_general(k, qm, _NT_DIMS, preferred_element_type=f32)
        s_refs[c][z_st, j * R:(j + 1) * R, :] = s
        mm = jnp.max(s.reshape(R // 8, 8, TQ), axis=0)
        return mm if m8 is None else jnp.maximum(m8, mm)

    z_st0 = z_ref[0]
    m8s = {}
    qms = {}
    for n in range(LAG):
        c, j = divmod(n, NP)
        if c not in qms:
            qms[c] = get_qm(jnp.int32(0), c)
        m8s[c] = stage_qk(z_st0, qms[c][0], qms[c][1], c, j, m8s.get(c))
    for c in m8s:
        m_ref[c] = m8s[c]
    ncarry = len(m8s)

    def head_body(h, carry):
        z_st = z_ref[0]
        z_ld = z_ref[1]
        h_next = jnp.minimum(h + 1, H - 1)
        w0 = pl.multiple_of((h * DH) // 8 * 8, 8)
        off = (h * DH) % 8
        rmask = (row >= off) & (row < off + DH)
        vt = vt_ref[pl.ds(w0, W), :]
        rm_full = jnp.concatenate([rmask] * (S // 128), axis=1)
        vth = jnp.where(rm_full, vt, jnp.ones_like(vt))
        rm_q = jnp.concatenate([rmask] * (TQ // 128), axis=1)
        m8s = {(0, c): m_ref[c] for c in range(ncarry)}
        qms = {}
        acc = None
        m = None
        for n in range(NT):
            dh, na = divmod(n + LAG, NT)
            ca, ja = divmod(na, NP)
            if (dh, ca) not in qms:
                qms[(dh, ca)] = get_qm(h_next if dh else h, ca)
            g, qm = qms[(dh, ca)]
            m8s[(dh, ca)] = stage_qk(z_st, g, qm, ca, ja, m8s.get((dh, ca)))
            c, j = divmod(n, NP)
            if j == 0:
                m = jnp.max(m8s[(0, c)], axis=0, keepdims=True)
                acc = None
            p = jnp.exp2(s_refs[c][z_ld, j * R:(j + 1) * R, :] - m).astype(bf16)
            o = jnp.dot(vth[:, j * R:(j + 1) * R], p, preferred_element_type=f32)
            acc = o if acc is None else acc + o
            if j == NP - 1:
                l = jnp.where(off == 0, acc[W - 1:W, :], acc[0:1, :])
                o = acc * pl.reciprocal(l, approx=False)
                pltpu.store(ot_ref.at[pl.ds(w0, W), c * TQ:(c + 1) * TQ], o, mask=rm_q)
        for c in range(ncarry):
            m_ref[c] = m8s[(1, c)]
        return carry

    jax.lax.fori_loop(0, H, head_body, 0)

    for c in w_copies[1:]:
        c.wait()

    def out_copy(i):
        return pltpu.make_async_copy(
            out_v.at[pl.ds(i * RB, RB), :], out_hbm.at[pl.ds(i * RB, RB), :], sem_o.at[i])

    def phase_c(i, carry):
        r0 = pl.multiple_of(i * RB, RB)
        o = ot_ref[:, pl.ds(r0, RB)].T.astype(bf16)
        hres = x_v[pl.ds(r0, RB), :].astype(f32) + jnp.dot(
            o, wo_v[...], preferred_element_type=f32)
        hn = _layernorm(hres).astype(bf16)
        a = jnp.dot(hn, w1_v[...], preferred_element_type=f32) + b1_v[...].astype(f32)
        a = _gelu(a).astype(bf16)
        y = jnp.dot(a, w2_v[...], preferred_element_type=f32) + b2_v[...].astype(f32)
        out_v[pl.ds(r0, RB), :] = (hres + y).astype(bf16)
        out_copy(i).start()
        return carry

    jax.lax.fori_loop(0, NB, phase_c, 0)
    for i in range(NB):
        out_copy(i).wait()


@jax.jit
def pallas_sequential_preLN__softmax_full_mha__dense_activation_gelu__prompt_kernel(
    A_x: jax.Array,
    A_wqkv: jax.Array,
    A_wo: jax.Array,
    B_x: jax.Array,
    B_w1: jax.Array,
    B_b1: jax.Array,
    B_w2: jax.Array,
    B_b2: jax.Array,
):
    del B_x
    bf16 = jnp.bfloat16
    f32 = jnp.float32
    x = A_x.reshape(S, D)
    b1 = B_b1.reshape(1, F)
    b2 = B_b2.reshape(1, D)
    any_spec = pl.BlockSpec(memory_space=pl.ANY)
    out = pl.pallas_call(
        _kernel,
        out_shape=jax.ShapeDtypeStruct((S, D), bf16),
        in_specs=[any_spec] * 7,
        out_specs=any_spec,
        scratch_shapes=[
            pltpu.VMEM((S, D), bf16),
            pltpu.VMEM((D, 3 * D), bf16),
            pltpu.VMEM((D, D), bf16),
            pltpu.VMEM((D, F), bf16),
            pltpu.VMEM((1, F), bf16),
            pltpu.VMEM((F, D), bf16),
            pltpu.VMEM((1, D), bf16),
            pltpu.VMEM((D, D), bf16),
            pltpu.VMEM((2 * NG - 1, S // 2, 128), jnp.uint32),
            pltpu.VMEM((2 * NG - 1, S // 2, 128), jnp.uint32),
            pltpu.VMEM((D, S), f32),
            pltpu.VMEM((D, S), f32),
            pltpu.VMEM((2, 8, TQ), f32),
            pltpu.VMEM((S, D), bf16),
            pltpu.SMEM((2,), jnp.int32),
            pltpu.SemaphoreType.DMA((NB,)),
            pltpu.SemaphoreType.DMA((6,)),
            pltpu.SemaphoreType.DMA((NB,)),
        ] + [pltpu.VMEM((1, S, TQ), f32)] * NQ,
        compiler_params=pltpu.CompilerParams(vmem_limit_bytes=100 * 1024 * 1024),
    )(x, A_wqkv, A_wo, B_w1, b1, B_w2, b2)
    return out.reshape(1, S, D)
```

```python
import functools
import math
import os

import jax
import jax.numpy as jnp
import jax.experimental.pallas as pl
import jax.experimental.pallas.tpu as pltpu

S = 2048
D = 640
F = 1536
H = 32
DH = D // H
NG = D // 128
EPS = 1e-5

TQ = 512
R = 128
NQ = S // TQ
NP = S // R
NT = NQ * NP
NTL = TQ // 128
SKEW = 2
LAG = NP + SKEW
W = 24
NPEEL = 2

NKV = int(os.environ.get('NKV', 160))
NKM = S - NKV
VT = int(os.environ.get('VT', 4))
_U16 = NKM // 16
SIZES = [(_U16 // NP + (1 if i < _U16 % NP else 0)) * 16 for i in range(NP)]
STARTS = [sum(SIZES[:i]) for i in range(NP)]
VUNITS = [(hf, b, d) for hf in range(16 // VT) for b in range(NKV // 8) for d in range(DH)]
NU = len(VUNITS)
BS = int(os.environ.get('BS', 4))
BSTEP = int(os.environ.get('BSTEP', 3))
PF32 = int(os.environ.get('PF32', 0))
ACCMEM = int(os.environ.get('ACCMEM', 1))
MMEM = int(os.environ.get('MMEM', 1))
PACE = 2

RB = 256
NB = S // RB

QSCALE = (DH ** -0.5) * math.log2(math.e)
NZ = 24
KW = (32, 48)


def _layernorm(x):
    m = jnp.mean(x, axis=-1, keepdims=True)
    xc = x - m
    v = jnp.mean(xc * xc, axis=-1, keepdims=True)
    return xc * jax.lax.rsqrt(v + EPS)


def _gelu(x):
    c = math.sqrt(2.0 / math.pi)
    return 0.5 * x * (1.0 + jnp.tanh(c * (x + 0.044715 * (x * x * x))))


def _kernel(x_hbm, wqkv_hbm, wo_hbm, w1_hbm, b1_hbm, w2_hbm, b2_hbm, out_hbm,
            x_v, wq_v, wk_v, wv_v, wo_v, w1_v, b1_v, w2_v, b2_v,
            xn_ref, kh_ref, qth_ref, qt_ref, va_ref, ot_ref, m_ref, hres_ref, hn_ref, out_v,
            z_ref, sem_in, sem_o,
            acc_ref, mb_ref, kf_ref, kb_a, kb_b, qb_a, qb_b, sv_a, sv_b, mv_a, mv_b, s0, s1, s2, s3):
    s_refs = (s0, s1, s2, s3)
    f32 = jnp.float32
    bf16 = jnp.bfloat16
    u32 = jnp.uint32

    def copy(src, dst, i):
        return pltpu.make_async_copy(src, dst, sem_in.at[i])

    def x_copy(r0, r1, i):
        return copy(x_hbm.at[0, r0:r1, :], x_v.at[r0:r1, :], i)

    x0a_c = x_copy(0, 256, 0)
    wql_c = copy(wqkv_hbm.at[:, 0:256], wq_v.at[:, 0:256], 1)
    x0b_c = x_copy(256, 512, 2)
    wqh_c = copy(wqkv_hbm.at[:, 256:D], wq_v.at[:, 256:D], 3)
    wk_c = copy(wqkv_hbm.at[:, D:2 * D], wk_v, 4)
    x1_c = x_copy(512, 1024, 5)
    wv_c = copy(wqkv_hbm.at[:, 2 * D:3 * D], wv_v, 6)
    x2_c = x_copy(1024, 2048, 7)
    late = [
        copy(wo_hbm, wo_v, 8),
        copy(w1_hbm, w1_v, 9),
        copy(w2_hbm, w2_v, 10),
        copy(b1_hbm, b1_v, 11),
        copy(b2_hbm, b2_v, 12),
    ]
    for c in [x0a_c, wql_c, x0b_c, wqh_c, wk_c, x1_c, wv_c, x2_c] + late:
        c.start()

    for i in range(NZ):
        z_ref[i] = 0

    def ln_a(r0, n):
        xn = _layernorm(x_v[r0:r0 + n, :].astype(f32)).astype(bf16)
        xn_ref[r0 // 2:(r0 + n) // 2, :] = pltpu.bitcast(xn, u32)

    pend = [[], []]

    def load_xn(r0, n):
        xp = xn_ref[r0 // 2:(r0 + n) // 2, :]
        toks = pend.pop(0)
        pend.append([])
        if toks:
            top = xp[0:8, 0:128]
            for i, tok in enumerate(toks):
                never = jnp.full((8, 128), z_ref[2 + i], jnp.int32) != 0
                top = jnp.where(never, pltpu.bitcast(tok, u32), top)
            xp = jnp.concatenate(
                [jnp.concatenate([top, xp[0:8, 128:]], axis=1), xp[8:]], axis=0)
        return pltpu.bitcast(xp, bf16)

    def store_q(q, r0, n):
        qt = q.astype(bf16).T
        qt_ref[:, r0:r0 + n] = qt.astype(f32)
        for h in range(H):
            w16 = (h // 2 * 2 * DH) // 16 * 16
            off = h * DH - w16
            kw = KW[h % 2]
            win = qt[w16:w16 + kw, :]
            row = jax.lax.broadcasted_iota(jnp.int32, (kw, n), 0)
            win = jnp.where((row >= off) & (row < off + DH), win, jnp.zeros_like(win))
            qth_ref[h, 0:kw // 2, r0:r0 + n] = pltpu.bitcast(win, u32)
        za = z_ref[1]
        pend[-1].append(qth_ref[za, 0:8, r0:r0 + 128])
        pend[-1].append(qt_ref[pl.ds(pl.multiple_of(za * 8, 8), 8), r0:r0 + 128])

    def q_part(r0, n, c0, c1):
        return jnp.dot(load_xn(r0, n), wq_v[:, c0:c1], preferred_element_type=f32) * QSCALE

    def mm_k(r0, n):
        return jnp.dot(load_xn(r0, n), wk_v[...], preferred_element_type=f32)

    def store_k(k, r0, n):
        kp = pltpu.bitcast(k.astype(bf16), u32)
        lane = jax.lax.broadcasted_iota(jnp.int32, (n // 2, 128), 1)
        gs = [kp[:, g * 128:(g + 1) * 128] for g in range(NG)]
        for hp in range(H // 2):
            w16 = (hp * 2 * DH) // 16 * 16
            g, lo = divmod(w16, 128)
            src = gs[g]
            if lo + 48 > 128:
                src = jnp.where(lane >= 64, gs[g], gs[g + 1])
            if lo:
                src = pltpu.roll(src, 128 - lo, 1)
            kh_ref[hp, r0 // 2:(r0 + n) // 2, :] = src
            if r0 + n == S:
                kf_ref[hp] = pltpu.bitcast(src[(n - NKV) // 2:], bf16).astype(f32)
        pend[-1].append(kh_ref[z_ref[1], r0 // 2:r0 // 2 + 8, :])

    def proj_q(r0, n):
        store_q(q_part(r0, n, 0, D), r0, n)

    def proj_k(r0, n):
        store_k(mm_k(r0, n), r0, n)

    def proj_v(r0, n):
        row_n = jax.lax.broadcasted_iota(jnp.int32, (W, n), 0)
        v = jnp.dot(load_xn(r0, n), wv_v[...], preferred_element_type=f32)
        vt = v.astype(bf16).T.astype(f32)
        for h in range(H):
            w0 = (h * DH) // 8 * 8
            off = (h * DH) % 8
            win = vt[w0:w0 + W, :]
            va_ref[h, :, r0:r0 + n] = jnp.where(
                (row_n >= off) & (row_n < off + DH), win, 1.0)
        pend[-1].append(va_ref[z_ref[1], 0:8, r0:r0 + 128])

    x0a_c.wait()
    ln_a(0, 256)
    wql_c.wait()
    x0b_c.wait()
    ql0 = q_part(0, 256, 0, 256)
    ln_a(256, 256)
    ql1 = q_part(256, 256, 0, 256)
    wqh_c.wait()
    qs = []
    for r0, ql in ((0, ql0), (256, ql1)):
        for u in range(2):
            qh = q_part(r0 + u * 128, 128, 256, D)
            qs.append(jnp.concatenate([ql[u * 128:(u + 1) * 128], qh], axis=1))
    store_q(qs[0], 0, 128)
    store_q(qs[1], 128, 128)
    wk_c.wait()
    store_q(qs[2], 256, 128)
    store_q(qs[3], 384, 128)
    proj_k(0, 128)
    proj_k(128, 128)
    k2 = mm_k(256, 128)
    k3 = mm_k(384, 128)
    x1_c.wait()
    wv_c.wait()
    store_k(k2, 256, 128)
    store_k(k3, 384, 128)
    ln_a(512, 256)
    proj_v(0, 256)
    ln_a(768, 256)
    proj_v(256, 256)
    proj_q(512, 256)
    q2 = q_part(768, 128, 0, D)
    q3 = q_part(896, 128, 0, D)
    x2_c.wait()
    store_q(q2, 768, 128)
    store_q(q3, 896, 128)
    ln_a(1024, 256)
    proj_k(512, 256)
    ln_a(1280, 256)
    proj_v(512, 256)
    proj_q(1024, 256)
    ln_a(1536, 256)
    proj_k(768, 256)
    proj_v(768, 256)
    proj_q(1280, 256)
    ln_a(1792, 256)
    proj_k(1024, 256)
    proj_v(1024, 256)
    proj_q(1536, 256)
    proj_k(1792, 256)
    proj_v(1280, 256)
    proj_q(1792, 256)
    proj_k(1280, 256)
    proj_v(1536, 256)
    proj_k(1536, 256)
    proj_v(1792, 256)

    row = jax.lax.broadcasted_iota(jnp.int32, (W, TQ), 0)

    class Z:
        def __init__(self):
            self.st = z_ref[0]
            self.ld = z_ref[1]
            self.q = [z_ref[2 + i] for i in range(NP)]
            self.never = [jnp.full((8, 128), z_ref[2 + NP + i], jnp.int32) != 0
                          for i in range(4)]
            self.zero = z_ref[0].astype(f32)

    def tie(never, tok, x):
        return jnp.where(never, tok, x)

    def qk(zs, h, par, c, r0, n, zq):
        kw = KW[par]
        k = pltpu.bitcast(kh_ref[h >> 1, r0 // 2:(r0 + n) // 2, :], bf16)[:, 0:kw]
        qm = pltpu.bitcast(qth_ref[h + zq, 0:kw // 2, c * TQ:(c + 1) * TQ], bf16)
        return jnp.dot(k, qm, preferred_element_type=f32)

    def max8(s):
        return jnp.max(s.reshape(s.shape[0] // 8, 8, s.shape[1]), axis=0)

    def stage_qk(zs, h, par, c, j, m8):
        r0, n = STARTS[j], SIZES[j]
        s = qk(zs, h, par, c, r0, n, zs.q[j])
        s_refs[c][zs.st, r0:r0 + n, :] = s
        mm = max8(s)
        return s, (mm if m8 is None else jnp.maximum(m8, mm))

    def mk_kb(zs, h, par, kb, d, tok=None):
        k = kf_ref[h >> 1]
        idx8 = jnp.full((8, 128), (((h >> 1) * 2 * DH) & 15) + (par * DH + d), jnp.int32)
        if tok is not None:
            idx8 = tie(zs.never[0], pltpu.bitcast(tok, jnp.int32), idx8)
        idx = jnp.concatenate([idx8] * (NKV // 8), axis=0)
        r = jnp.take_along_axis(k, idx, axis=1)
        kb[zs.st, d] = r
        return kb[zs.ld, d, 0:8, :]

    def mk_qb(zs, h, par, qb, t, tok=None):
        w0 = pl.multiple_of((h * DH) // 8 * 8, 8)
        off = 4 * par
        win = qt_ref[pl.ds(w0, W), t * 128:(t + 1) * 128]
        if tok is not None:
            win = jnp.concatenate(
                [tie(zs.never[0], tok, win[g * 8:(g + 1) * 8]) for g in range(W // 8)], axis=0)
        last = None
        for d in range(DH):
            last = jnp.broadcast_to(win[off + d:off + d + 1, :], (8, 128))
            qb[zs.st, d, :, t * 128:(t + 1) * 128] = last
        return qb[zs.ld, 0, :, t * 128:(t + 1) * 128]

    zs0 = Z()
    h0 = jnp.int32(0) + zs0.st
    for d in range(DH):
        mk_kb(zs0, h0 + 1, 1, kb_b, d)
    for t in range(S // 128):
        mk_qb(zs0, h0 + 1, 1, qb_b, t)
    for c in range(NQ):
        s = qk(zs0, h0, 0, c, NKM, NKV, zs0.q[c])
        sv_a[zs0.st, :, c * TQ:(c + 1) * TQ] = s
        mv_a[zs0.st, :, c * TQ:(c + 1) * TQ] = max8(s)
    m8s = {}
    for n in range(LAG):
        c, j = divmod(n, NP)
        _, m8s[c] = stage_qk(zs0, h0, 0, c, j, m8s.get(c))
    for c in m8s:
        m_ref[c] = m8s[c]
    ncarry = len(m8s)

    def head(zs, h, par, m8_in, hist, build=True, last=False, filler=None):
        kbs, qbs, svs, mvs = (kb_a, kb_b), (qb_a, qb_b), (sv_a, sv_b), (mv_a, mv_b)
        sv_cur, mv_cur = svs[par], mvs[par]
        sv_nxt, mv_nxt, kb_r, qb_r = svs[1 - par], mvs[1 - par], kbs[1 - par], qbs[1 - par]
        kb_w, qb_w = kbs[par], qbs[par]
        w0 = pl.multiple_of((h * DH) // 8 * 8, 8)
        off = 4 * par
        rmask = (row >= off) & (row < off + DH)
        never4 = [jnp.concatenate([nv] * NTL, axis=1) for nv in zs.never]
        m8s = {(0, c): m8_in[c] for c in range(ncarry)}
        acc = None
        m = None
        vacc = None
        extra = {}
        nv_steps = NT - 2
        for n in range(NT):
            dh, na = divmod(n + LAG, NT)
            ca, ja = divmod(na, NP)
            if dh and last:
                filler(na)
                hist = []
            else:
                s, m8s[(dh, ca)] = stage_qk(zs, h + dh, (par + dh) % 2, ca, ja, m8s.get((dh, ca)))
                stok = s_refs[ca][zs.ld, STARTS[ja]:STARTS[ja] + 8, 0:128]
                hist.append((s, m8s[(dh, ca)], stok))
            if not last and n < nv_steps:
                us = list(range(n * NU // nv_steps, (n + 1) * NU // nv_steps))
                pt = [s[i * 8:(i + 1) * 8, t * 128:(t + 1) * 128]
                      for i in range(s.shape[0] // 8) for t in (0, 2)]
                for iu, u in enumerate(us):
                    hf, b, d = VUNITS[u]
                    kk = tie(zs.never[0], pt[iu * len(pt) // len(us)],
                             kb_r[zs.ld, d, b * 8:(b + 1) * 8, :])
                    if d == 0:
                        vacc = [None] * VT
                    for t in range(VT):
                        col = (hf * VT + t) * 128
                        pr = kk * qb_r[zs.ld, d, :, col:col + 128]
                        vacc[t] = pr if vacc[t] is None else vacc[t] + pr
                    if d == DH - 1:
                        cols = slice(hf * VT * 128, (hf + 1) * VT * 128)
                        res = jnp.concatenate(vacc, axis=1)
                        sv_nxt[zs.st, b * 8:(b + 1) * 8, cols] = res
                        if b > 0:
                            res = jnp.maximum(res, mv_nxt[zs.ld, :, cols])
                        mv_nxt[zs.st, :, cols] = res
            if build:
                if n % 3 == 0 and n // 3 < DH:
                    extra[n + 3] = mk_kb(zs, h + 2, par, kb_w, n // 3, s[0:8, 0:128])
                if n % 3 == 1 and n // 3 < S // 128:
                    extra[n + 3] = mk_qb(zs, h + 2, par, qb_w, n // 3, s[0:8, 0:128])
            c, j = divmod(n, NP)
            if j == 0:
                mm8 = jnp.maximum(m8s[(0, c)], mv_cur[zs.ld, :, c * TQ:(c + 1) * TQ])
                m = jnp.broadcast_to(jnp.max(mm8, axis=0, keepdims=True), (8, TQ))
                if MMEM:
                    mb_ref[zs.st] = m
            me = mb_ref[zs.q[j]] if MMEM else m
            if len(hist) > PACE:
                me = tie(never4[1], hist[-1 - PACE][1], me)
                me = jnp.concatenate(
                    [me[:, 0:128], tie(zs.never[2], hist[-1 - PACE][2], me[:, 128:256]),
                     me[:, 256:]], axis=1)
            if n in extra:
                me = jnp.concatenate(
                    [tie(zs.never[3], extra[n], me[:, 0:128]), me[:, 128:]], axis=1)
            lo_r, hi_r = j * R, (j + 1) * R
            parts = []
            if lo_r < NKM:
                parts.append(s_refs[c][zs.ld, lo_r:min(hi_r, NKM), :])
            if hi_r > NKM:
                parts.append(sv_cur[zs.ld, max(lo_r - NKM, 0):hi_r - NKM, c * TQ:(c + 1) * TQ])
            sv = jnp.concatenate(parts, axis=0) if len(parts) > 1 else parts[0]
            rows = R // BS
            outs = [None] * BS
            for kk in range(BS):
                part = BS - 1 - kk
                mek = me
                if len(hist) >= 2:
                    i0 = BSTEP * kk * 8
                    tk = hist[-2][0][i0:i0 + 8, 0:128]
                    mek = tie(never4[0], jnp.concatenate([tk] * NTL, axis=1), me)
                outs[part] = jnp.exp2(
                    sv[part * rows:(part + 1) * rows].reshape(rows // 8, 8, TQ) - mek[None])
            p = jnp.concatenate(outs, axis=0).reshape(R, TQ)
            if not PF32:
                p = p.astype(bf16)
            o = jnp.dot(va_ref[h, :, j * R:(j + 1) * R], p, preferred_element_type=f32)
            if ACCMEM:
                acc = o if j == 0 else acc_ref[zs.ld] + o
                if j < NP - 1:
                    acc_ref[zs.st] = acc
            else:
                acc = (jnp.full((W, TQ), zs.zero, f32) + o) if j == 0 else acc + o
            if j == NP - 1:
                l = acc[0:1, :] if par else acc[W - 1:W, :]
                o = acc * pl.reciprocal(l, approx=False)
                pltpu.store(ot_ref.at[pl.ds(w0, W), c * TQ:(c + 1) * TQ], o, mask=rmask)
        if last:
            return None
        return [m8s[(1, c)] for c in range(ncarry)]

    def heads_body(i, carry):
        zs = Z()
        m8 = [m_ref[c] for c in range(ncarry)]
        hist = []
        for u in range(2):
            m8 = head(zs, i * 2 + u, u, m8, hist)
        for c in range(ncarry):
            m_ref[c] = m8[c]
        return carry

    NLOOP = (H - NPEEL) // 2
    jax.lax.fori_loop(0, NLOOP, heads_body, 0)

    for c in late:
        c.wait()

    def out_copy(i):
        return pltpu.make_async_copy(
            out_v.at[pl.ds(i * RB, RB), :], out_hbm.at[0, pl.ds(i * RB, RB), :], sem_o.at[i])

    def get_o(i):
        r0 = pl.multiple_of(i * RB, RB)
        return ot_ref[:, pl.ds(r0, RB)].T.astype(bf16)

    def attn_out(i, o):
        r0 = pl.multiple_of(i * RB, RB)
        r0h = pl.multiple_of(i * (RB // 2), RB // 2)
        hres = x_v[pl.ds(r0, RB), :].astype(f32) + jnp.dot(
            o, wo_v[...], preferred_element_type=f32)
        hres_ref[pl.ds(r0, RB), :] = hres
        hn_ref[pl.ds(r0h, RB // 2), :] = pltpu.bitcast(_layernorm(hres).astype(bf16), u32)

    def ffn1(i):
        r0h = pl.multiple_of(i * (RB // 2), RB // 2)
        hn = pltpu.bitcast(hn_ref[pl.ds(r0h, RB // 2), :], bf16)
        a = jnp.dot(hn, w1_v[...], preferred_element_type=f32) + b1_v[...].astype(f32)[None, :]
        return _gelu(a).astype(bf16)

    def ffn2(i, a):
        r0 = pl.multiple_of(i * RB, RB)
        y = jnp.dot(a, w2_v[...], preferred_element_type=f32) + b2_v[...].astype(f32)[None, :]
        out_v[pl.ds(r0, RB), :] = (hres_ref[pl.ds(r0, RB), :] + y).astype(bf16)
        out_copy(i).start()

    st = {}

    def filler(na):
        if na == 0:
            st['o'] = get_o(0)
            st['y'] = []
        if na % 3 == 2 and na // 3 < NG:
            g = na // 3
            st['y'].append(jnp.dot(st['o'], wo_v[:, g * 128:(g + 1) * 128],
                                   preferred_element_type=f32))
        if na == LAG - 1:
            hres = x_v[0:RB, :].astype(f32) + jnp.concatenate(st['y'], axis=1)
            hres_ref[0:RB, :] = hres
            hn_ref[0:RB // 2, :] = pltpu.bitcast(_layernorm(hres).astype(bf16), u32)

    zs = Z()
    m8 = [m_ref[c] for c in range(ncarry)]
    hist = []
    for u in range(NPEEL):
        hh = jnp.int32(H - NPEEL + u) + zs.st
        m8 = head(zs, hh, u, m8, hist, build=False, last=(u == NPEEL - 1), filler=filler)

    def phase_c(i, carry):
        o = get_o(i + 1)
        a = ffn1(i)
        attn_out(i + 1, o)
        ffn2(i, a)
        return carry

    jax.lax.fori_loop(0, NB - 1, phase_c, 0)
    ffn2(NB - 1, ffn1(NB - 1))
    for i in range(NB):
        out_copy(i).wait()


@jax.jit
def pallas_sequential_preLN__softmax_full_mha__dense_activation_gelu__prompt_kernel(
    A_x: jax.Array,
    A_wqkv: jax.Array,
    A_wo: jax.Array,
    B_x: jax.Array,
    B_w1: jax.Array,
    B_b1: jax.Array,
    B_w2: jax.Array,
    B_b2: jax.Array,
):
    del B_x
    bf16 = jnp.bfloat16
    f32 = jnp.float32
    u32 = jnp.uint32
    any_spec = pl.BlockSpec(memory_space=pl.ANY)
    return pl.pallas_call(
        _kernel,
        out_shape=jax.ShapeDtypeStruct((1, S, D), bf16),
        in_specs=[any_spec] * 7,
        out_specs=any_spec,
        scratch_shapes=[
            pltpu.VMEM((S, D), bf16),
            pltpu.VMEM((D, D), bf16),
            pltpu.VMEM((D, D), bf16),
            pltpu.VMEM((D, D), bf16),
            pltpu.VMEM((D, D), bf16),
            pltpu.VMEM((D, F), bf16),
            pltpu.VMEM((F,), bf16),
            pltpu.VMEM((F, D), bf16),
            pltpu.VMEM((D,), bf16),
            pltpu.VMEM((S // 2, D), u32),
            pltpu.VMEM((H // 2, S // 2, 128), u32),
            pltpu.VMEM((H, 24, S), u32),
            pltpu.VMEM((D, S), f32),
            pltpu.VMEM((H, W, S), f32),
            pltpu.VMEM((D, S), f32),
            pltpu.VMEM((2, 8, TQ), f32),
            pltpu.VMEM((S, D), f32),
            pltpu.VMEM((S // 2, D), u32),
            pltpu.VMEM((S, D), bf16),
            pltpu.SMEM((NZ,), jnp.int32),
            pltpu.SemaphoreType.DMA((13,)),
            pltpu.SemaphoreType.DMA((NB,)),
            pltpu.VMEM((1, W, TQ), f32),
            pltpu.VMEM((1, 8, TQ), f32),
            pltpu.VMEM((H // 2, NKV, 128), f32),
        ] + [pltpu.VMEM((1, DH, NKV, 128), f32)] * 2
          + [pltpu.VMEM((1, DH, 8, S), f32)] * 2
          + [pltpu.VMEM((1, NKV, S), f32)] * 2
          + [pltpu.VMEM((1, 8, S), f32)] * 2
          + [pltpu.VMEM((1, NKM, TQ), f32)] * NQ,
        compiler_params=pltpu.CompilerParams(vmem_limit_bytes=110 * 1024 * 1024),
    )(A_x, A_wqkv, A_wo, B_w1, B_b1, B_w2, B_b2)
```

```python
import math

import jax
import jax.numpy as jnp
import jax.experimental.pallas as pl
import jax.experimental.pallas.tpu as pltpu

S = 2048
D = 640
F = 1536
H = 32
DH = D // H
NG = D // 128
EPS = 1e-5

TQ = 512
R = 128
NQ = S // TQ
NP = S // R
NT = NQ * NP
NTL = TQ // 128
W = 24
NPEEL = 2

NKV = 224
NKM = S - NKV
VT = 8
VUNITS = [(hf, b, d) for hf in range(16 // VT) for b in range(NKV // 8) for d in range(DH)]
NU = len(VUNITS)
_U16 = NKM // 16
SIZES = [(_U16 // NP + (1 if i < _U16 % NP else 0)) * 16 for i in range(NP)]
STARTS = [NKV + sum(SIZES[:i]) for i in range(NP)]
LEAD = 2
T0 = NT // 4
SAFE_L = 2.0 ** 60
SAFE_ACC = 2.0 ** 120

RB = 256
NB = S // RB

QSCALE = (DH ** -0.5) * math.log2(math.e)
NZ = 24
KW = (32, 48)


def _layernorm(x):
    m = jnp.mean(x, axis=-1, keepdims=True)
    xc = x - m
    v = jnp.mean(xc * xc, axis=-1, keepdims=True)
    return xc * jax.lax.rsqrt(v + EPS)


def _gelu(x):
    c = math.sqrt(2.0 / math.pi)
    return 0.5 * x * (1.0 + jnp.tanh(c * (x + 0.044715 * (x * x * x))))


def _kernel(x_hbm, wqkv_hbm, wo_hbm, w1_hbm, b1_hbm, w2_hbm, b2_hbm, out_hbm,
            x_v, wq_v, wk_v, wv_v, wo_v, w1_v, w2_v,
            xn_ref, kh_ref, qth_ref, qt_ref, va_ref, ot_ref, hres_ref, hn_ref, out_v,
            z_ref, sem_in, sem_o,
            acc_ref, chk_ref, kf_ref, kb_a, kb_b, qb_a, qb_b, sv_a, sv_b, mv_a, mv_b,
            mb_a, mb_b, qa_a, qa_b, *rest):
    p_refs, (b1_v, b2_v) = rest[:NP], rest[NP:]
    f32 = jnp.float32
    bf16 = jnp.bfloat16
    u32 = jnp.uint32

    def copy(src, dst, i):
        return pltpu.make_async_copy(src, dst, sem_in.at[i])

    def x_copy(r0, r1, i):
        return copy(x_hbm.at[0, r0:r1, :], x_v.at[r0:r1, :], i)

    x0a_c = x_copy(0, 256, 0)
    wql_c = copy(wqkv_hbm.at[:, 0:256], wq_v.at[:, 0:256], 1)
    x0b_c = x_copy(256, 512, 2)
    wqh_c = copy(wqkv_hbm.at[:, 256:D], wq_v.at[:, 256:D], 3)
    wk_c = copy(wqkv_hbm.at[:, D:2 * D], wk_v, 4)
    x1_c = x_copy(512, 1024, 5)
    wv_c = copy(wqkv_hbm.at[:, 2 * D:3 * D], wv_v, 6)
    x2_c = x_copy(1024, 2048, 7)
    late = [
        copy(wo_hbm, wo_v, 8),
        copy(w1_hbm, w1_v, 9),
        copy(w2_hbm, w2_v, 10),
        copy(b1_hbm, b1_v, 11),
        copy(b2_hbm, b2_v, 12),
    ]
    for c in [x0a_c, wql_c, x0b_c, wqh_c, wk_c, x1_c, wv_c, x2_c] + late:
        c.start()

    for i in range(NZ):
        z_ref[i] = 0

    def pack16(x):
        n, m = x.shape
        x = x.reshape(n // 16, 2, 8, m)
        pk = pltpu.pack_elementwise([x[:, 0], x[:, 1]], packed_dtype=bf16)
        pk = pk.reshape(n // 2, m)
        return pk if pk.dtype == u32 else pltpu.bitcast(pk, u32)

    def ln_a(r0, n):
        xn = _layernorm(x_v[r0:r0 + n, :].astype(f32)).astype(bf16)
        xn_ref[r0 // 2:(r0 + n) // 2, :] = pltpu.bitcast(xn, u32)

    pend = [[], []]

    def load_xn(r0, n):
        xp = xn_ref[r0 // 2:(r0 + n) // 2, :]
        toks = pend.pop(0)
        pend.append([])
        if toks:
            top = xp[0:8, 0:128]
            for i, tok in enumerate(toks):
                never = jnp.full((8, 128), z_ref[2 + i], jnp.int32) != 0
                top = jnp.where(never, pltpu.bitcast(tok, u32), top)
            xp = jnp.concatenate(
                [jnp.concatenate([top, xp[0:8, 128:]], axis=1), xp[8:]], axis=0)
        return pltpu.bitcast(xp, bf16)

    def store_q(q, r0, n):
        qt = q.astype(bf16).T.astype(f32)
        qt_ref[:, r0:r0 + n] = qt
        for h in range(H):
            par = h % 2
            w0 = h // 2 * 2 * DH
            zero8 = jnp.zeros((8, n), f32)
            row = jax.lax.broadcasted_iota(jnp.int32, (40, n), 0)
            win = jnp.where((row >= par * DH) & (row < (par + 1) * DH), qt[w0:w0 + 40, :], 0.0)
            win = jnp.concatenate([zero8, win], axis=0).astype(bf16)
            qth_ref[h, :, r0:r0 + n] = pltpu.bitcast(win, u32)
        za = z_ref[1]
        pend[-1].append(qth_ref[za, 0:8, r0:r0 + 128])
        pend[-1].append(qt_ref[pl.ds(pl.multiple_of(za * 8, 8), 8), r0:r0 + 128])

    def q_part(r0, n, c0, c1):
        return jnp.dot(load_xn(r0, n), wq_v[:, c0:c1], preferred_element_type=f32) * QSCALE

    def mm_k(r0, n):
        return jnp.dot(load_xn(r0, n), wk_v[...], preferred_element_type=f32)

    def store_k(k, r0, n):
        kp = pltpu.bitcast(k.astype(bf16), u32)
        lane = jax.lax.broadcasted_iota(jnp.int32, (n // 2, 128), 1)
        gs = [kp[:, g * 128:(g + 1) * 128] for g in range(NG)]
        ones = jnp.full((n // 2, 128), 0x3F803F80, u32)
        for hp in range(H // 2):
            g, lo = divmod(hp * 2 * DH, 128)
            src = gs[g]
            if lo + 2 * DH > 128:
                src = jnp.where(lane >= 64, gs[g], gs[g + 1])
            if lo != 8:
                src = pltpu.roll(src, (8 - lo) % 128, 1)
            src = jnp.where(lane < 8, ones, src)
            kh_ref[hp, r0 // 2:(r0 + n) // 2, :] = src
            if r0 < NKV:
                nk = min(n, NKV - r0)
                kf_ref[hp, r0:r0 + nk] = pltpu.bitcast(src[0:nk // 2], bf16).astype(f32)
        pend[-1].append(kh_ref[z_ref[1], r0 // 2:r0 // 2 + 8, :])

    def proj_q(r0, n):
        store_q(q_part(r0, n, 0, D), r0, n)

    def proj_k(r0, n):
        store_k(mm_k(r0, n), r0, n)

    def proj_v(r0, n):
        row_n = jax.lax.broadcasted_iota(jnp.int32, (W, n), 0)
        v = jnp.dot(load_xn(r0, n), wv_v[...], preferred_element_type=f32)
        vt = pltpu.bitcast(pack16(v), bf16).T.astype(f32)
        for h in range(H):
            w0 = (h * DH) // 8 * 8
            off = (h * DH) % 8
            win = vt[w0:w0 + W, :]
            va_ref[h, :, r0:r0 + n] = jnp.where(
                (row_n >= off) & (row_n < off + DH), win, 1.0)
        pend[-1].append(va_ref[z_ref[1], 0:8, r0:r0 + 128])

    row = jax.lax.broadcasted_iota(jnp.int32, (W, TQ), 0)

    class Z:
        def __init__(self):
            self.st = z_ref[0]
            self.ld = z_ref[1]
            self.q = [z_ref[2 + i] for i in range(NP)]
            self.never = [jnp.full((8, 128), z_ref[2 + NP + i], jnp.int32) != 0
                          for i in range(2)]

    def tie(never, tok, x):
        return jnp.where(never, tok, x)

    def max8(s):
        return jnp.max(s.reshape(s.shape[0] // 8, 8, s.shape[1]), axis=0)

    def load_k(h, par, r0, n):
        return pltpu.bitcast(kh_ref[h >> 1, r0 // 2:(r0 + n) // 2, :], bf16)[:, 0:KW[par]]

    def mk_kb(zs, h, par, kb, d, tok=None):
        k = kf_ref[h >> 1, 0:NKV]
        idx8 = jnp.full((8, 128), 8 + par * DH + d, jnp.int32)
        if tok is not None:
            idx8 = tie(zs.never[0], pltpu.bitcast(tok, jnp.int32), idx8)
        idx = jnp.concatenate([idx8] * (NKV // 8), axis=0)
        kb[zs.st, d] = jnp.take_along_axis(k, idx, axis=1)
        return kb[zs.ld, d, 0:8, :]

    def mk_qb(zs, h, par, qb, t, tok=None):
        w0 = (h * DH) // 8 * 8 if isinstance(h, int) else pl.multiple_of((h * DH) // 8 * 8, 8)
        off = 4 * par
        win = qt_ref[pl.ds(w0, W), t * 128:(t + 1) * 128]
        if tok is not None:
            win = jnp.concatenate(
                [tie(zs.never[0], tok, win[g * 8:(g + 1) * 8]) for g in range(W // 8)], axis=0)
        for d in range(DH):
            qb[zs.st, d, :, t * 128:(t + 1) * 128] = jnp.broadcast_to(
                win[off + d:off + d + 1, :], (8, 128))
        return qb[zs.ld, 0, :, t * 128:(t + 1) * 128]

    kbs, qbs, svs, mvs = (kb_a, kb_b), (qb_a, qb_b), (sv_a, sv_b), (mv_a, mv_b)
    mbs, qas = (mb_a, mb_b), (qa_a, qa_b)
    row8 = jax.lax.broadcasted_iota(jnp.int32, (8, TQ), 0)

    def set_qa(zs, h, par, c):
        m = jnp.max(mvs[par][zs.ld, :, c * TQ:(c + 1) * TQ], axis=0, keepdims=True)
        m = jnp.broadcast_to(m.astype(bf16).astype(f32), (8, TQ))
        mbs[c % 2][zs.st] = m
        q = qth_ref[h, :, c * TQ:(c + 1) * TQ]
        neg = jax.lax.shift_right_logical(pltpu.bitcast(-m, u32), jnp.uint32(16))
        top = jnp.where(row8 == 0, neg, q[0:8])
        qas[c % 2][zs.st] = jnp.concatenate([top, q[8:]], axis=0)

    def store_p(zs, r0, p):
        n = p.shape[0]
        a = r0
        while a < r0 + n:
            t = a // R
            b = min(r0 + n, (t + 1) * R)
            p_refs[t][zs.st, (a - t * R) // 2:(b - t * R) // 2, :] = pack16(p[a - r0:b - r0])
            a = b

    def stage_qk(zs, h, par, c, j):
        qm = pltpu.bitcast(qas[c % 2][zs.q[j], 0:KW[par] // 2, :], bf16)
        s = jnp.dot(load_k(h, par, STARTS[j], SIZES[j]), qm,
                    preferred_element_type=f32)
        store_p(zs, STARTS[j], jnp.exp2(s))
        return s

    def stage_vexp(zs, par, c, g, zq, tok=None):
        sv = svs[par][zs.ld, g * 16:(g + 1) * 16, c * TQ:(c + 1) * TQ].reshape(2, 8, TQ)
        m = mbs[c % 2][zq]
        if tok is not None:
            m = tie(jnp.concatenate([zs.never[0]] * NTL, axis=1),
                    jnp.concatenate([tok] * NTL, axis=1), m)
        store_p(zs, g * 16, jnp.exp2(sv - m[None]).reshape(16, TQ))

    x0a_c.wait()
    ln_a(0, 256)
    wql_c.wait()
    x0b_c.wait()
    ql0 = q_part(0, 256, 0, 256)
    ln_a(256, 256)
    ql1 = q_part(256, 256, 0, 256)
    wqh_c.wait()
    qs = []
    for r0, ql in ((0, ql0), (256, ql1)):
        for u in range(2):
            qh = q_part(r0 + u * 128, 128, 256, D)
            qs.append(jnp.concatenate([ql[u * 128:(u + 1) * 128], qh], axis=1))
    store_q(qs[0], 0, 128)
    store_q(qs[1], 128, 128)
    wk_c.wait()
    store_q(qs[2], 256, 128)
    store_q(qs[3], 384, 128)
    proj_k(0, 128)
    proj_k(128, 128)
    k2 = mm_k(256, 128)
    k3 = mm_k(384, 128)
    x1_c.wait()
    wv_c.wait()
    store_k(k2, 256, 128)
    store_k(k3, 384, 128)
    ln_a(512, 256)
    proj_v(0, 256)
    ln_a(768, 256)
    proj_v(256, 256)
    proj_q(512, 256)
    q2 = q_part(768, 128, 0, D)
    q3 = q_part(896, 128, 0, D)
    x2_c.wait()
    store_q(q2, 768, 128)
    store_q(q3, 896, 128)
    zs0 = Z()
    h0 = 0
    chk_ref[...] = jnp.zeros(chk_ref.shape, f32)

    def pre_kb(d0, d1):
        for d in range(d0, d1):
            tok = mk_kb(zs0, h0, 0, kb_a, d)
        pend[-1].append(tok)
        for d in range(d0, d1):
            tok = mk_kb(zs0, 1, 1, kb_b, d)
        pend[-1].append(tok)

    def pre_qb(t0, t1):
        for t in range(t0, t1):
            tok = mk_qb(zs0, h0, 0, qb_a, t)
        pend[-1].append(tok)
        for t in list(range(t0, t1)) + list(range(t0 - 8, t1 - 8)):
            tok = mk_qb(zs0, 1, 1, qb_b, t)
        pend[-1].append(tok)

    def pre_sv(c, nk=NKV):
        qm = pltpu.bitcast(qth_ref[h0, 0:KW[0] // 2, c * TQ:(c + 1) * TQ], bf16)
        s = jnp.dot(load_k(h0, 0, 0, nk), qm, preferred_element_type=f32)
        sv_a[zs0.st, 0:nk, c * TQ:(c + 1) * TQ] = s
        mv_a[zs0.st, :, c * TQ:(c + 1) * TQ] = max8(s)

    ln_a(1024, 256)
    proj_k(512, 256)
    ln_a(1280, 256)
    proj_v(512, 256)
    pre_kb(0, 4)
    proj_q(1024, 256)
    ln_a(1536, 256)
    proj_k(768, 256)
    proj_v(768, 256)
    pre_kb(4, 8)
    pre_qb(8, 10)
    proj_q(1280, 256)
    ln_a(1792, 256)
    proj_k(1024, 256)
    proj_v(1024, 256)
    pre_kb(8, 12)
    pre_qb(10, 12)
    proj_q(1536, 256)
    proj_k(1792, 256)
    proj_v(1280, 256)
    pre_kb(12, 16)
    pre_qb(12, 14)
    proj_q(1792, 256)
    proj_k(1280, 256)
    pre_kb(16, 20)
    proj_v(1536, 256)
    pre_qb(14, 16)
    proj_k(1536, 256)
    pre_sv(0)
    proj_v(1792, 256)
    set_qa(zs0, h0, 0, 0)
    for g in range(NKV // 16):
        stage_vexp(zs0, 0, 0, g, zs0.ld)
    pre_sv(1)
    pre_sv(2, NKV // 2)
    pre_sv(3, NKV // 2)
    for n in range(LEAD):
        stage_qk(zs0, h0, 0, 0, n)

    def normalize(zs, h, par, c, acc):
        w0 = pl.multiple_of((h * DH) // 8 * 8, 8)
        off = 4 * par
        l = acc[0:1, :] if par else acc[W - 1:W, :]
        rl = pl.reciprocal(l, approx=False)
        chk_ref[0] = jnp.maximum(chk_ref[0], jnp.broadcast_to(jnp.maximum(l, rl), (8, TQ)))
        chk_ref[1] = jnp.maximum(chk_ref[1], max8(jnp.abs(acc)))
        o = acc * rl
        pltpu.store(ot_ref.at[pl.ds(w0, W), c * TQ:(c + 1) * TQ], o,
                    mask=(row >= off) & (row < off + DH))

    def head(zs, h, par, last=False, filler=None, build=True):
        vacc = None
        extra = {}
        extra2 = {}
        ng = NKV // 16
        j0 = -(-NKV // R) + 1
        for n in range(NT):
            dh, na = divmod(n + LEAD, NT)
            ca, ja = divmod(na, NP)
            c, j = divmod(n, NP)
            s = None
            if last:
                filler(n)
            if not (dh and last):
                s = stage_qk(zs, h + dh, (par + dh) % 2, ca, ja)
            dn, cn = divmod(c + 1, NQ)
            if not (dn and last):
                if j == j0 - 1:
                    set_qa(zs, h + dn, (par + dn) % 2, cn)
                if j0 <= j < NP - 1:
                    k0, k1 = (j - j0) * ng // (NP - 1 - j0), (j + 1 - j0) * ng // (NP - 1 - j0)
                    for g in range(k0, k1):
                        i0 = (g - k0) * 48 + 24
                        stage_vexp(zs, (par + dn) % 2, cn, g, zs.q[j], s[i0:i0 + 8, 0:128])
            if not (last and n >= T0):
                vp = par if n < T0 else 1 - par
                sv_w, mv_w, kb_r, qb_r = svs[vp], mvs[vp], kbs[vp], qbs[vp]
                nn = (n - T0) % NT
                us = list(range(nn * NU // NT, (nn + 1) * NU // NT))
                pt = [s[i * 8:(i + 1) * 8, t * 128:(t + 1) * 128]
                      for i in range(s.shape[0] // 8) for t in range(NTL)]
                for iu, u in enumerate(us):
                    hf, b, d = VUNITS[u]
                    kk = tie(zs.never[0], pt[iu * len(pt) // len(us)],
                             kb_r[zs.ld, d, b * 8:(b + 1) * 8, :])
                    if d == 0:
                        vacc = [None] * VT
                    for t in range(VT):
                        col = (hf * VT + t) * 128
                        pr = kk * qb_r[zs.q[b % 4], d, :, col:col + 128]
                        vacc[t] = pr if vacc[t] is None else vacc[t] + pr
                    if d == DH - 1:
                        cols = slice(hf * VT * 128, (hf + 1) * VT * 128)
                        res = jnp.concatenate(vacc, axis=1)
                        sv_w[zs.st, b * 8:(b + 1) * 8, cols] = res
                        if b > 0:
                            res = jnp.maximum(res, mv_w[zs.ld, :, cols])
                        mv_w[zs.st, :, cols] = res
            bn = n - T0 - 2
            if build and bn >= 0:
                if bn % 2 == 0 and bn // 2 < DH:
                    extra[n + 3] = mk_kb(zs, h + 2, par, kbs[par], bn // 2, s[0:8, 0:128])
                if bn % 2 == 1 and bn // 2 < S // 128:
                    extra2[n + 3] = mk_qb(zs, h + 2, par, qbs[par], bn // 2, s[64:72, 0:128])
            v = va_ref[h, :, j * R:(j + 1) * R]
            if n in extra:
                v = jnp.concatenate([tie(zs.never[1], extra[n], v[0:8]), v[8:]], axis=0)
            if n in extra2:
                v = jnp.concatenate(
                    [v[0:8], tie(zs.never[1], extra2[n], v[8:16]), v[16:]], axis=0)
            o = jnp.dot(v, pltpu.bitcast(p_refs[j][zs.ld], bf16), preferred_element_type=f32)
            acc = o if j == 0 else acc_ref[zs.ld] + o
            if j < NP - 1:
                acc_ref[zs.st] = acc
            else:
                normalize(zs, h, par, c, acc)

    def heads_body(i, carry):
        zs = Z()
        for u in range(2):
            head(zs, i * 2 + u, u)
        return carry

    NLOOP = (H - NPEEL) // 2
    jax.lax.fori_loop(0, NLOOP, heads_body, 0)

    for c in late:
        c.wait()

    def out_copy(i):
        return pltpu.make_async_copy(
            out_v.at[pl.ds(i * RB, RB), :], out_hbm.at[0, pl.ds(i * RB, RB), :], sem_o.at[i])

    def get_o(i):
        r0 = pl.multiple_of(i * RB, RB)
        return ot_ref[:, pl.ds(r0, RB)].T.astype(bf16)

    def attn_out(i, o):
        r0 = pl.multiple_of(i * RB, RB)
        r0h = pl.multiple_of(i * (RB // 2), RB // 2)
        hres = x_v[pl.ds(r0, RB), :].astype(f32) + jnp.dot(
            o, wo_v[...], preferred_element_type=f32)
        hres_ref[pl.ds(r0, RB), :] = hres
        hn_ref[pl.ds(r0h, RB // 2), :] = pltpu.bitcast(_layernorm(hres).astype(bf16), u32)

    def ffn1(i):
        r0h = pl.multiple_of(i * (RB // 2), RB // 2)
        hn = pltpu.bitcast(hn_ref[pl.ds(r0h, RB // 2), :], bf16)
        a = jnp.dot(hn, w1_v[...], preferred_element_type=f32) + b1_v[...].astype(f32)[None, :]
        return _gelu(a).astype(bf16)

    def ffn2(i, a):
        r0 = pl.multiple_of(i * RB, RB)
        y = jnp.dot(a, w2_v[...], preferred_element_type=f32) + b2_v[...].astype(f32)[None, :]
        out_v[pl.ds(r0, RB), :] = (hres_ref[pl.ds(r0, RB), :] + y).astype(bf16)
        out_copy(i).start()

    st = {}

    def filler(n):
        k = n - (NT - 14)
        if k == 0:
            st['o'] = get_o(0)
            st['y'] = []
        if k >= 2 and k % 2 == 0 and (k - 2) // 2 < NG:
            g = (k - 2) // 2
            st['y'].append(jnp.dot(st['o'], wo_v[:, g * 128:(g + 1) * 128],
                                   preferred_element_type=f32))
        if k == 11:
            hres = x_v[0:RB, :].astype(f32) + jnp.concatenate(st['y'], axis=1)
            hres_ref[0:RB, :] = hres
            hn_ref[0:RB // 2, :] = pltpu.bitcast(_layernorm(hres).astype(bf16), u32)

    zs = Z()
    for u in range(NPEEL):
        hh = jnp.int32(H - NPEEL + u) + zs.st
        head(zs, hh, u, last=(u == NPEEL - 1), filler=filler, build=False)

    safe = jnp.logical_and(jnp.max(chk_ref[0]) < SAFE_L, jnp.max(chk_ref[1]) < SAFE_ACC)

    @pl.when(jnp.logical_not(safe))
    def _():
        def exact(i, carry):
            h = i // NQ
            c0 = pl.multiple_of((i % NQ) * TQ, TQ)
            k = pltpu.bitcast(kh_ref[h >> 1], bf16)[:, 0:KW[1]]
            qm = pltpu.bitcast(qth_ref[h, :, pl.ds(c0, TQ)], bf16)
            s = jnp.dot(k, qm, preferred_element_type=f32)
            p = jnp.exp2(s - jnp.max(s, axis=0, keepdims=True))
            acc = jnp.dot(va_ref[h], pltpu.bitcast(pack16(p), bf16),
                          preferred_element_type=f32)
            w0 = pl.multiple_of((h * DH) // 8 * 8, 8)
            off = (h * DH) % 8
            l = jnp.where(off == 0, acc[W - 1:W, :], acc[0:1, :])
            pltpu.store(ot_ref.at[pl.ds(w0, W), pl.ds(c0, TQ)], acc / l,
                        mask=(row >= off) & (row < off + DH))
            return carry

        jax.lax.fori_loop(0, H * NQ, exact, 0)
        attn_out(0, get_o(0))

    def c_step(i):
        o = get_o(i + 1)
        a = ffn1(i)
        attn_out(i + 1, o)
        ffn2(i, a)

    def phase_c(i, carry):
        c_step(2 * i)
        c_step(2 * i + 1)
        return carry

    jax.lax.fori_loop(0, (NB - 2) // 2, phase_c, 0)
    zc = z_ref[0]
    c_step(NB - 2 + zc)
    ffn2(NB - 1 + zc, ffn1(NB - 1 + zc))
    for i in range(NB):
        out_copy(i).wait()


@jax.jit
def pallas_sequential_preLN__softmax_full_mha__dense_activation_gelu__prompt_kernel(
    A_x: jax.Array,
    A_wqkv: jax.Array,
    A_wo: jax.Array,
    B_x: jax.Array,
    B_w1: jax.Array,
    B_b1: jax.Array,
    B_w2: jax.Array,
    B_b2: jax.Array,
):
    del B_x
    bf16 = jnp.bfloat16
    f32 = jnp.float32
    u32 = jnp.uint32
    any_spec = pl.BlockSpec(memory_space=pl.ANY)
    return pl.pallas_call(
        _kernel,
        out_shape=jax.ShapeDtypeStruct((1, S, D), bf16),
        in_specs=[any_spec] * 7,
        out_specs=any_spec,
        scratch_shapes=[
            pltpu.VMEM((S, D), bf16),
            pltpu.VMEM((D, D), bf16),
            pltpu.VMEM((D, D), bf16),
            pltpu.VMEM((D, D), bf16),
            pltpu.VMEM((D, D), bf16),
            pltpu.VMEM((D, F), bf16),
            pltpu.VMEM((F, D), bf16),
            pltpu.VMEM((S // 2, D), u32),
            pltpu.VMEM((H // 2, S // 2, 128), u32),
            pltpu.VMEM((H, 24, S), u32),
            pltpu.VMEM((D, S), f32),
            pltpu.VMEM((H, W, S), f32),
            pltpu.VMEM((D, S), f32),
            pltpu.VMEM((S, D), f32),
            pltpu.VMEM((S // 2, D), u32),
            pltpu.VMEM((S, D), bf16),
            pltpu.SMEM((NZ,), jnp.int32),
            pltpu.SemaphoreType.DMA((13,)),
            pltpu.SemaphoreType.DMA((NB,)),
            pltpu.VMEM((1, W, TQ), f32),
            pltpu.VMEM((2, 8, TQ), f32),
            pltpu.VMEM((H // 2, -(-NKV // 32) * 32, 128), f32),
        ] + [pltpu.VMEM((1, DH, NKV, 128), f32)] * 2
          + [pltpu.VMEM((1, DH, 8, S), f32)] * 2
          + [pltpu.VMEM((1, NKV, S), f32)] * 2
          + [pltpu.VMEM((1, 8, S), f32)] * 2
          + [pltpu.VMEM((1, 8, TQ), f32)] * 2
          + [pltpu.VMEM((1, 24, TQ), u32)] * 2
          + [pltpu.VMEM((1, R // 2, TQ), u32)] * NP
          + [pltpu.VMEM((F,), bf16), pltpu.VMEM((D,), bf16)],
        compiler_params=pltpu.CompilerParams(vmem_limit_bytes=110 * 1024 * 1024),
    )(A_x, A_wqkv, A_wo, B_w1, B_b1, B_w2, B_b2)
```

```python
import math

import jax
import jax.numpy as jnp
import jax.experimental.pallas as pl
import jax.experimental.pallas.tpu as pltpu

S = 2048
D = 640
F = 1536
H = 32
DH = D // H
NG = D // 128
EPS = 1e-5

TQ = 512
R = 128
NQ = S // TQ
NP = S // R
NT = NQ * NP
NTL = TQ // 128
W = 24
NPEEL = 2

NKV = 224
NKM = S - NKV
VT = 8
VUNITS = [(hf, b, d) for hf in range(16 // VT) for b in range(NKV // 8) for d in range(DH)]
NU = len(VUNITS)
_U16 = NKM // 16
SIZES = [(_U16 // NP + (1 if i < _U16 % NP else 0)) * 16 for i in range(NP)]
STARTS = [NKV + sum(SIZES[:i]) for i in range(NP)]
LEAD = 2
T0 = NT // 4
SAFE_L = 2.0 ** 60
SAFE_ACC = 2.0 ** 120

RB = 256
NB = S // RB

QSCALE = (DH ** -0.5) * math.log2(math.e)
NZ = 24
KW = (32, 48)


def _layernorm(x):
    m = jnp.mean(x, axis=-1, keepdims=True)
    xc = x - m
    v = jnp.mean(xc * xc, axis=-1, keepdims=True)
    return xc * jax.lax.rsqrt(v + EPS)


def _gelu(x):
    c = math.sqrt(2.0 / math.pi)
    return 0.5 * x * (1.0 + jnp.tanh(c * (x + 0.044715 * (x * x * x))))


def _kernel(x_hbm, wqkv_hbm, wo_hbm, w1_hbm, b1_hbm, w2_hbm, b2_hbm, out_hbm,
            x_v, wq_v, wk_v, wv_v, wo_v, w1_v, w2_v,
            xn_ref, kh_ref, qth_ref, qt_ref, va_ref, ot_ref, hres_ref, hn_ref, out_v,
            z_ref, sem_in, sem_o,
            acc_ref, chk_ref, kf_ref, kb_a, kb_b, qb_a, qb_b, sv_a, sv_b, mv_a, mv_b,
            mb_a, mb_b, qa_a, qa_b, *rest):
    p_refs, (b1_v, b2_v) = rest[:NP], rest[NP:]
    f32 = jnp.float32
    bf16 = jnp.bfloat16
    u32 = jnp.uint32

    def copy(src, dst, i):
        return pltpu.make_async_copy(src, dst, sem_in.at[i])

    def x_copy(r0, r1, i):
        return copy(x_hbm.at[0, r0:r1, :], x_v.at[r0:r1, :], i)

    x0a_c = x_copy(0, 256, 0)
    wql_c = copy(wqkv_hbm.at[:, 0:256], wq_v.at[:, 0:256], 1)
    x0b_c = x_copy(256, 512, 2)
    wqh_c = copy(wqkv_hbm.at[:, 256:D], wq_v.at[:, 256:D], 3)
    wk_c = copy(wqkv_hbm.at[:, D:2 * D], wk_v, 4)
    x1_c = x_copy(512, 1024, 5)
    wv_c = copy(wqkv_hbm.at[:, 2 * D:3 * D], wv_v, 6)
    x2_c = x_copy(1024, 2048, 7)
    late = [
        copy(wo_hbm, wo_v, 8),
        copy(w1_hbm, w1_v, 9),
        copy(w2_hbm, w2_v, 10),
        copy(b1_hbm, b1_v, 11),
        copy(b2_hbm, b2_v, 12),
    ]
    for c in [x0a_c, wql_c, x0b_c, wqh_c, wk_c, x1_c, wv_c, x2_c] + late:
        c.start()

    for i in range(NZ):
        z_ref[i] = 0

    def ln_a(r0, n):
        xn = _layernorm(x_v[r0:r0 + n, :].astype(f32)).astype(bf16)
        xn_ref[r0 // 2:(r0 + n) // 2, :] = pltpu.bitcast(xn, u32)

    pend = [[], []]

    def load_xn(r0, n):
        xp = xn_ref[r0 // 2:(r0 + n) // 2, :]
        toks = pend.pop(0)
        pend.append([])
        if toks:
            top = xp[0:8, 0:128]
            for i, tok in enumerate(toks):
                never = jnp.full((8, 128), z_ref[2 + i], jnp.int32) != 0
                top = jnp.where(never, pltpu.bitcast(tok, u32), top)
            xp = jnp.concatenate(
                [jnp.concatenate([top, xp[0:8, 128:]], axis=1), xp[8:]], axis=0)
        return pltpu.bitcast(xp, bf16)

    def store_q(q, r0, n):
        qt = q.astype(bf16).T.astype(f32)
        qt_ref[:, r0:r0 + n] = qt
        for h in range(H):
            par = h % 2
            w0 = h // 2 * 2 * DH
            zero8 = jnp.zeros((8, n), f32)
            row = jax.lax.broadcasted_iota(jnp.int32, (40, n), 0)
            win = jnp.where((row >= par * DH) & (row < (par + 1) * DH), qt[w0:w0 + 40, :], 0.0)
            win = jnp.concatenate([zero8, win], axis=0).astype(bf16)
            qth_ref.at[h][:, r0:r0 + n] = pltpu.bitcast(win, u32)
        za = z_ref[1]
        pend[-1].append(qth_ref[za, 0:8, r0:r0 + 128])
        pend[-1].append(qt_ref[pl.ds(pl.multiple_of(za * 8, 8), 8), r0:r0 + 128])

    def q_part(r0, n, c0, c1):
        return jnp.dot(load_xn(r0, n), wq_v[:, c0:c1], preferred_element_type=f32) * QSCALE

    def mm_k(r0, n):
        return jnp.dot(load_xn(r0, n), wk_v[...], preferred_element_type=f32)

    def store_k(k, r0, n):
        kp = pltpu.bitcast(k.astype(bf16), u32)
        lane = jax.lax.broadcasted_iota(jnp.int32, (n // 2, 128), 1)
        gs = [kp[:, g * 128:(g + 1) * 128] for g in range(NG)]
        ones = jnp.full((n // 2, 128), 0x3F803F80, u32)
        for hp in range(H // 2):
            g, lo = divmod(hp * 2 * DH, 128)
            src = gs[g]
            if lo + 2 * DH > 128:
                src = jnp.where(lane >= 64, gs[g], gs[g + 1])
            if lo != 8:
                src = pltpu.roll(src, (8 - lo) % 128, 1)
            src = jnp.where(lane < 8, ones, src)
            kh_ref[hp, r0 // 2:(r0 + n) // 2, :] = src
            if r0 < NKV:
                nk = min(n, NKV - r0)
                kf_ref[hp, r0:r0 + nk] = pltpu.bitcast(src[0:nk // 2], bf16).astype(f32)
        pend[-1].append(kh_ref[z_ref[1], r0 // 2:r0 // 2 + 8, :])

    def proj_q(r0, n):
        store_q(q_part(r0, n, 0, D), r0, n)

    def proj_k(r0, n):
        store_k(mm_k(r0, n), r0, n)

    def proj_v(r0, n):
        row_n = jax.lax.broadcasted_iota(jnp.int32, (W, n), 0)
        v = jnp.dot(load_xn(r0, n), wv_v[...], preferred_element_type=f32)
        vt = v.astype(bf16).T.astype(f32)
        for h in range(H):
            w0 = (h * DH) // 8 * 8
            off = (h * DH) % 8
            win = vt[w0:w0 + W, :]
            va_ref[h, :, r0:r0 + n] = jnp.where(
                (row_n >= off) & (row_n < off + DH), win, 1.0)
        pend[-1].append(va_ref[z_ref[1], 0:8, r0:r0 + 128])

    row = jax.lax.broadcasted_iota(jnp.int32, (W, TQ), 0)

    class Z:
        def __init__(self):
            self.st = z_ref[0]
            self.ld = z_ref[1]
            self.q = [z_ref[2 + i] for i in range(NP)]
            self.never = [jnp.full((8, 128), z_ref[2 + NP + i], jnp.int32) != 0
                          for i in range(2)]

    def tie(never, tok, x):
        return jnp.where(never, tok, x)

    def max8(s):
        return jnp.max(s.reshape(s.shape[0] // 8, 8, s.shape[1]), axis=0)

    def load_k(h, par, r0, n):
        return pltpu.bitcast(kh_ref[h >> 1, r0 // 2:(r0 + n) // 2, :], bf16)[:, 0:KW[par]]

    def mk_kb(zs, h, par, kb, d, tok=None):
        k = kf_ref[h >> 1, 0:NKV]
        idx8 = jnp.full((8, 128), 8 + par * DH + d, jnp.int32)
        if tok is not None:
            idx8 = tie(zs.never[0], pltpu.bitcast(tok, jnp.int32), idx8)
        idx = jnp.concatenate([idx8] * (NKV // 8), axis=0)
        kb[zs.st, d] = jnp.take_along_axis(k, idx, axis=1)
        return kb[zs.ld, d, 0:8, :]

    def mk_qb(zs, h, par, qb, t, tok=None):
        w0 = (h * DH) // 8 * 8 if isinstance(h, int) else pl.multiple_of((h * DH) // 8 * 8, 8)
        off = 4 * par
        win = qt_ref[pl.ds(w0, W), t * 128:(t + 1) * 128]
        if tok is not None:
            win = jnp.concatenate(
                [tie(zs.never[0], tok, win[g * 8:(g + 1) * 8]) for g in range(W // 8)], axis=0)
        for d in range(DH):
            qb[zs.st, d, :, t * 128:(t + 1) * 128] = jnp.broadcast_to(
                win[off + d:off + d + 1, :], (8, 128))
        return qb[zs.ld, 0, :, t * 128:(t + 1) * 128]

    kbs, qbs, svs, mvs = (kb_a, kb_b), (qb_a, qb_b), (sv_a, sv_b), (mv_a, mv_b)
    mbs, qas = (mb_a, mb_b), (qa_a, qa_b)
    row8 = jax.lax.broadcasted_iota(jnp.int32, (8, TQ), 0)

    def set_qa(zs, h, par, c):
        m = jnp.max(mvs[par][zs.ld, :, c * TQ:(c + 1) * TQ], axis=0, keepdims=True)
        m = jnp.broadcast_to(m.astype(bf16).astype(f32), (8, TQ))
        mbs[c % 2][zs.st] = m
        q = qth_ref[h, :, c * TQ:(c + 1) * TQ]
        neg = jax.lax.shift_right_logical(pltpu.bitcast(-m, u32), jnp.uint32(16))
        top = jnp.where(row8 == 0, neg, q[0:8])
        qas[c % 2][zs.st] = jnp.concatenate([top, q[8:]], axis=0)

    def store_p(zs, r0, p):
        n = p.shape[0]
        a = r0
        while a < r0 + n:
            t = a // R
            b = min(r0 + n, (t + 1) * R)
            p_refs[t].at[zs.st][(a - t * R) // 2:(b - t * R) // 2, :] = pltpu.bitcast(
                p[a - r0:b - r0].astype(bf16), u32)
            a = b

    def stage_qk(zs, h, par, c, j):
        qm = pltpu.bitcast(qas[c % 2][zs.q[j], 0:KW[par] // 2, :], bf16)
        s = jnp.dot(load_k(h, par, STARTS[j], SIZES[j]), qm,
                    preferred_element_type=f32)
        store_p(zs, STARTS[j], jnp.exp2(s))
        return s

    def stage_vexp(zs, par, c, g, zq, tok=None):
        sv = svs[par][zs.ld, g * 16:(g + 1) * 16, c * TQ:(c + 1) * TQ]
        m = mbs[c % 2][zq]
        if tok is not None:
            m = tie(jnp.concatenate([zs.never[0]] * NTL, axis=1),
                    jnp.concatenate([tok] * NTL, axis=1), m)
        store_p(zs, g * 16, jnp.exp2(sv - jnp.concatenate([m, m], axis=0)))

    x0a_c.wait()
    ln_a(0, 256)
    wql_c.wait()
    x0b_c.wait()
    ql0 = q_part(0, 256, 0, 256)
    ln_a(256, 256)
    ql1 = q_part(256, 256, 0, 256)
    wqh_c.wait()
    qs = []
    for r0, ql in ((0, ql0), (256, ql1)):
        for u in range(2):
            qh = q_part(r0 + u * 128, 128, 256, D)
            qs.append(jnp.concatenate([ql[u * 128:(u + 1) * 128], qh], axis=1))
    store_q(qs[0], 0, 128)
    store_q(qs[1], 128, 128)
    wk_c.wait()
    store_q(qs[2], 256, 128)
    store_q(qs[3], 384, 128)
    proj_k(0, 128)
    proj_k(128, 128)
    k2 = mm_k(256, 128)
    k3 = mm_k(384, 128)
    x1_c.wait()
    wv_c.wait()
    store_k(k2, 256, 128)
    store_k(k3, 384, 128)
    ln_a(512, 256)
    proj_v(0, 256)
    ln_a(768, 256)
    proj_v(256, 256)
    proj_q(512, 256)
    q2 = q_part(768, 128, 0, D)
    q3 = q_part(896, 128, 0, D)
    x2_c.wait()
    store_q(q2, 768, 128)
    store_q(q3, 896, 128)
    zs0 = Z()
    h0 = 0
    chk_ref[...] = jnp.zeros(chk_ref.shape, f32)

    def pre_kb(d0, d1):
        for d in range(d0, d1):
            tok = mk_kb(zs0, h0, 0, kb_a, d)
        pend[-1].append(tok)
        for d in range(d0, d1):
            tok = mk_kb(zs0, 1, 1, kb_b, d)
        pend[-1].append(tok)

    def pre_qb(t0, t1):
        for t in range(t0, t1):
            tok = mk_qb(zs0, h0, 0, qb_a, t)
        pend[-1].append(tok)
        for t in list(range(t0, t1)) + list(range(t0 - 8, t1 - 8)):
            tok = mk_qb(zs0, 1, 1, qb_b, t)
        pend[-1].append(tok)

    def pre_sv(c, nk=NKV):
        qm = pltpu.bitcast(qth_ref[h0, 0:KW[0] // 2, c * TQ:(c + 1) * TQ], bf16)
        s = jnp.dot(load_k(h0, 0, 0, nk), qm, preferred_element_type=f32)
        sv_a[zs0.st, 0:nk, c * TQ:(c + 1) * TQ] = s
        mv_a[zs0.st, :, c * TQ:(c + 1) * TQ] = max8(s)

    ln_a(1024, 256)
    proj_k(512, 256)
    ln_a(1280, 256)
    proj_v(512, 256)
    pre_kb(0, 4)
    proj_q(1024, 256)
    ln_a(1536, 256)
    proj_k(768, 256)
    proj_v(768, 256)
    pre_kb(4, 8)
    pre_qb(8, 10)
    proj_q(1280, 256)
    ln_a(1792, 256)
    proj_k(1024, 256)
    proj_v(1024, 256)
    pre_kb(8, 12)
    pre_qb(10, 12)
    proj_q(1536, 256)
    proj_k(1792, 256)
    proj_v(1280, 256)
    pre_kb(12, 16)
    pre_qb(12, 14)
    proj_q(1792, 256)
    proj_k(1280, 256)
    pre_kb(16, 20)
    proj_v(1536, 256)
    pre_qb(14, 16)
    proj_k(1536, 256)
    pre_sv(0)
    proj_v(1792, 256)
    set_qa(zs0, h0, 0, 0)
    for g in range(NKV // 16):
        stage_vexp(zs0, 0, 0, g, zs0.ld)
    pre_sv(1)
    pre_sv(2, NKV // 2)
    pre_sv(3, NKV // 2)
    for n in range(LEAD):
        stage_qk(zs0, h0, 0, 0, n)

    def normalize(zs, h, par, c, acc):
        w0 = pl.multiple_of((h * DH) // 8 * 8, 8)
        off = 4 * par
        l = acc[0:1, :] if par else acc[W - 1:W, :]
        rl = pl.reciprocal(l, approx=False)
        chk_ref[0] = jnp.maximum(chk_ref[0], jnp.broadcast_to(jnp.maximum(l, rl), (8, TQ)))
        chk_ref[1] = jnp.maximum(chk_ref[1], max8(jnp.abs(acc)))
        o = acc * rl
        pltpu.store(ot_ref.at[pl.ds(w0, W), c * TQ:(c + 1) * TQ], o,
                    mask=(row >= off) & (row < off + DH))

    def head(zs, h, par, last=False, filler=None, build=True):
        vacc = None
        extra = {}
        extra2 = {}
        ng = NKV // 16
        j0 = -(-NKV // R) + 1
        for n in range(NT):
            dh, na = divmod(n + LEAD, NT)
            ca, ja = divmod(na, NP)
            c, j = divmod(n, NP)
            s = None
            if last:
                filler(n)
            if not (dh and last):
                s = stage_qk(zs, h + dh, (par + dh) % 2, ca, ja)
            dn, cn = divmod(c + 1, NQ)
            if not (dn and last):
                if j == j0 - 1:
                    set_qa(zs, h + dn, (par + dn) % 2, cn)
                if j0 <= j < NP - 1:
                    k0, k1 = (j - j0) * ng // (NP - 1 - j0), (j + 1 - j0) * ng // (NP - 1 - j0)
                    for g in range(k0, k1):
                        i0 = (g - k0) * 48 + 24
                        stage_vexp(zs, (par + dn) % 2, cn, g, zs.q[j], s[i0:i0 + 8, 0:128])
            if not (last and n >= T0):
                vp = par if n < T0 else 1 - par
                sv_w, mv_w, kb_r, qb_r = svs[vp], mvs[vp], kbs[vp], qbs[vp]
                nn = (n - T0) % NT
                us = list(range(nn * NU // NT, (nn + 1) * NU // NT))
                npt = s.shape[0] // 8 * NTL
                for iu, u in enumerate(us):
                    hf, b, d = VUNITS[u]
                    cols = slice(hf * VT * 128, (hf + 1) * VT * 128)
                    ti, tt = divmod(iu * npt // len(us), NTL)
                    kk = tie(zs.never[0], s[ti * 8:(ti + 1) * 8, tt * 128:(tt + 1) * 128],
                             kb_r[zs.ld, d, b * 8:(b + 1) * 8, :])
                    pr = jnp.concatenate([kk] * VT, axis=1) * qb_r[zs.q[b % 4], d, :, cols]
                    vacc = pr if d == 0 else vacc + pr
                    if d == DH - 1:
                        res = vacc
                        sv_w[zs.st, b * 8:(b + 1) * 8, cols] = res
                        if b > 0:
                            res = jnp.maximum(res, mv_w[zs.ld, :, cols])
                        mv_w[zs.st, :, cols] = res
            bn = n - T0 - 2
            if build and bn >= 0:
                if bn % 2 == 0 and bn // 2 < DH:
                    extra[n + 3] = mk_kb(zs, h + 2, par, kbs[par], bn // 2, s[0:8, 0:128])
                if bn % 2 == 1 and bn // 2 < S // 128:
                    extra2[n + 3] = mk_qb(zs, h + 2, par, qbs[par], bn // 2, s[64:72, 0:128])
            v = va_ref[h, :, j * R:(j + 1) * R]
            if n in extra:
                v = jnp.concatenate([tie(zs.never[1], extra[n], v[0:8]), v[8:]], axis=0)
            if n in extra2:
                v = jnp.concatenate(
                    [v[0:8], tie(zs.never[1], extra2[n], v[8:16]), v[16:]], axis=0)
            o = jnp.dot(v, pltpu.bitcast(p_refs[j][zs.ld], bf16), preferred_element_type=f32)
            acc = o if j == 0 else acc_ref[zs.ld] + o
            if j < NP - 1:
                acc_ref[zs.st] = acc
            else:
                normalize(zs, h, par, c, acc)

    def heads_body(i, carry):
        zs = Z()
        for u in range(2):
            head(zs, i * 2 + u, u)
        return carry

    NLOOP = (H - NPEEL) // 2
    jax.lax.fori_loop(0, NLOOP, heads_body, 0)

    for c in late:
        c.wait()

    def out_copy(i):
        return pltpu.make_async_copy(
            out_v.at[pl.ds(i * RB, RB), :], out_hbm.at[0, pl.ds(i * RB, RB), :], sem_o.at[i])

    def get_o(i):
        r0 = pl.multiple_of(i * RB, RB)
        return ot_ref[:, pl.ds(r0, RB)].T.astype(bf16)

    def attn_out(i, o):
        r0 = pl.multiple_of(i * RB, RB)
        r0h = pl.multiple_of(i * (RB // 2), RB // 2)
        hres = x_v[pl.ds(r0, RB), :].astype(f32) + jnp.dot(
            o, wo_v[...], preferred_element_type=f32)
        hres_ref[pl.ds(r0, RB), :] = hres
        hn_ref[pl.ds(r0h, RB // 2), :] = pltpu.bitcast(_layernorm(hres).astype(bf16), u32)

    def ffn1(i):
        r0h = pl.multiple_of(i * (RB // 2), RB // 2)
        hn = pltpu.bitcast(hn_ref[pl.ds(r0h, RB // 2), :], bf16)
        a = jnp.dot(hn, w1_v[...], preferred_element_type=f32) + b1_v[...].astype(f32)[None, :]
        return _gelu(a).astype(bf16)

    def ffn2(i, a):
        r0 = pl.multiple_of(i * RB, RB)
        y = jnp.dot(a, w2_v[...], preferred_element_type=f32) + b2_v[...].astype(f32)[None, :]
        out_v[pl.ds(r0, RB), :] = (hres_ref[pl.ds(r0, RB), :] + y).astype(bf16)
        out_copy(i).start()

    st = {}

    def filler(n):
        k = n - (NT - 14)
        if k == 0:
            st['o'] = get_o(0)
            st['y'] = []
        if k >= 2 and k % 2 == 0 and (k - 2) // 2 < NG:
            g = (k - 2) // 2
            st['y'].append(jnp.dot(st['o'], wo_v[:, g * 128:(g + 1) * 128],
                                   preferred_element_type=f32))
        if k == 11:
            hres = x_v[0:RB, :].astype(f32) + jnp.concatenate(st['y'], axis=1)
            hres_ref[0:RB, :] = hres
            hn_ref[0:RB // 2, :] = pltpu.bitcast(_layernorm(hres).astype(bf16), u32)

    zs = Z()
    for u in range(NPEEL):
        hh = jnp.int32(H - NPEEL + u) + zs.st
        head(zs, hh, u, last=(u == NPEEL - 1), filler=filler, build=False)

    safe = jnp.logical_and(jnp.max(chk_ref[0]) < SAFE_L, jnp.max(chk_ref[1]) < SAFE_ACC)

    @pl.when(jnp.logical_not(safe))
    def _():
        def exact(i, carry):
            h = i // NQ
            c0 = pl.multiple_of((i % NQ) * TQ, TQ)
            k = pltpu.bitcast(kh_ref[h >> 1], bf16)[:, 0:KW[1]]
            qm = pltpu.bitcast(qth_ref[h, :, pl.ds(c0, TQ)], bf16)
            s = jnp.dot(k, qm, preferred_element_type=f32)
            p = jnp.exp2(s - jnp.max(s, axis=0, keepdims=True))
            acc = jnp.dot(va_ref[h], p.astype(bf16), preferred_element_type=f32)
            w0 = pl.multiple_of((h * DH) // 8 * 8, 8)
            off = (h * DH) % 8
            l = jnp.where(off == 0, acc[W - 1:W, :], acc[0:1, :])
            pltpu.store(ot_ref.at[pl.ds(w0, W), pl.ds(c0, TQ)], acc / l,
                        mask=(row >= off) & (row < off + DH))
            return carry

        jax.lax.fori_loop(0, H * NQ, exact, 0)
        attn_out(0, get_o(0))

    def c_step(i):
        o = get_o(i + 1)
        a = ffn1(i)
        attn_out(i + 1, o)
        ffn2(i, a)

    def phase_c(i, carry):
        c_step(2 * i)
        c_step(2 * i + 1)
        return carry

    jax.lax.fori_loop(0, (NB - 2) // 2, phase_c, 0)
    zc = z_ref[0]
    c_step(NB - 2 + zc)
    ffn2(NB - 1 + zc, ffn1(NB - 1 + zc))
    for i in range(NB):
        out_copy(i).wait()


@jax.jit
def pallas_sequential_preLN__softmax_full_mha__dense_activation_gelu__prompt_kernel(
    A_x: jax.Array,
    A_wqkv: jax.Array,
    A_wo: jax.Array,
    B_x: jax.Array,
    B_w1: jax.Array,
    B_b1: jax.Array,
    B_w2: jax.Array,
    B_b2: jax.Array,
):
    del B_x
    bf16 = jnp.bfloat16
    f32 = jnp.float32
    u32 = jnp.uint32
    any_spec = pl.BlockSpec(memory_space=pl.ANY)
    return pl.pallas_call(
        _kernel,
        out_shape=jax.ShapeDtypeStruct((1, S, D), bf16),
        in_specs=[any_spec] * 7,
        out_specs=any_spec,
        scratch_shapes=[
            pltpu.VMEM((S, D), bf16),
            pltpu.VMEM((D, D), bf16),
            pltpu.VMEM((D, D), bf16),
            pltpu.VMEM((D, D), bf16),
            pltpu.VMEM((D, D), bf16),
            pltpu.VMEM((D, F), bf16),
            pltpu.VMEM((F, D), bf16),
            pltpu.VMEM((S // 2, D), u32),
            pltpu.VMEM((H // 2, S // 2, 128), u32),
            pltpu.VMEM((H, 24, S), u32),
            pltpu.VMEM((D, S), f32),
            pltpu.VMEM((H, W, S), f32),
            pltpu.VMEM((D, S), f32),
            pltpu.VMEM((S, D), f32),
            pltpu.VMEM((S // 2, D), u32),
            pltpu.VMEM((S, D), bf16),
            pltpu.SMEM((NZ,), jnp.int32),
            pltpu.SemaphoreType.DMA((13,)),
            pltpu.SemaphoreType.DMA((NB,)),
            pltpu.VMEM((1, W, TQ), f32),
            pltpu.VMEM((2, 8, TQ), f32),
            pltpu.VMEM((H // 2, -(-NKV // 32) * 32, 128), f32),
        ] + [pltpu.VMEM((1, DH, NKV, 128), f32)] * 2
          + [pltpu.VMEM((1, DH, 8, S), f32)] * 2
          + [pltpu.VMEM((1, NKV, S), f32)] * 2
          + [pltpu.VMEM((1, 8, S), f32)] * 2
          + [pltpu.VMEM((1, 8, TQ), f32)] * 2
          + [pltpu.VMEM((1, 24, TQ), u32)] * 2
          + [pltpu.VMEM((1, R // 2, TQ), u32)] * NP
          + [pltpu.VMEM((F,), bf16), pltpu.VMEM((D,), bf16)],
        compiler_params=pltpu.CompilerParams(vmem_limit_bytes=110 * 1024 * 1024),
    )(A_x, A_wqkv, A_wo, B_w1, B_b1, B_w2, B_b2)
```

```python
import math

import jax
import jax.numpy as jnp
import jax.experimental.pallas as pl
import jax.experimental.pallas.tpu as pltpu

S = 2048
D = 640
F = 1536
H = 32
DH = D // H
NG = D // 128
EPS = 1e-5

TQ = 512
R = 128
NQ = S // TQ
NP = S // R
NT = NQ * NP
NTL = TQ // 128
W = 24
NPEEL = 2

NKV = 224
NKM = S - NKV
VT = 8
VUNITS = [(hf, b, d) for hf in range(16 // VT) for b in range(NKV // 8) for d in range(DH)]
NU = len(VUNITS)
_U16 = NKM // 16
SIZES = [(_U16 // NP + (1 if i < _U16 % NP else 0)) * 16 for i in range(NP)]
STARTS = [NKV + sum(SIZES[:i]) for i in range(NP)]
LEAD = 2
T0 = NT // 4
SAFE_L = 2.0 ** 60
SAFE_ACC = 2.0 ** 120

RB = 256
NB = S // RB

QSCALE = (DH ** -0.5) * math.log2(math.e)
NZ = 24
KW = (32, 48)


def _layernorm(x):
    m = jnp.mean(x, axis=-1, keepdims=True)
    xc = x - m
    v = jnp.mean(xc * xc, axis=-1, keepdims=True)
    return xc * jax.lax.rsqrt(v + EPS)


def _gelu(x):
    c = math.sqrt(2.0 / math.pi)
    return 0.5 * x * (1.0 + jnp.tanh(c * (x + 0.044715 * (x * x * x))))


def _kernel(x_hbm, wqkv_hbm, wo_hbm, w1_hbm, b1_hbm, w2_hbm, b2_hbm, out_hbm,
            x_v, wq_v, wk_v, wv_v, wo_v, w1_v, w2_v,
            xn_ref, kh_ref, qth_ref, qt_ref, va_ref, ot_ref, hres_ref, hn_ref, out_v,
            z_ref, sem_in, sem_o,
            acc_ref, chk_ref, kf_ref, kb_a, kb_b, qb_a, qb_b, sv_a, sv_b, mv_a, mv_b,
            mb_a, mb_b, qa_a, qa_b, *rest):
    p_refs, (b1_v, b2_v) = rest[:NP], rest[NP:]
    f32 = jnp.float32
    bf16 = jnp.bfloat16
    u32 = jnp.uint32

    def copy(src, dst, i):
        return pltpu.make_async_copy(src, dst, sem_in.at[i])

    def x_copy(r0, r1, i):
        return copy(x_hbm.at[0, r0:r1, :], x_v.at[r0:r1, :], i)

    x0a_c = x_copy(0, 256, 0)
    wql_c = copy(wqkv_hbm.at[:, 0:256], wq_v.at[:, 0:256], 1)
    x0b_c = x_copy(256, 512, 2)
    wqh_c = copy(wqkv_hbm.at[:, 256:D], wq_v.at[:, 256:D], 3)
    wk_c = copy(wqkv_hbm.at[:, D:2 * D], wk_v, 4)
    x1_c = x_copy(512, 1024, 5)
    wv_c = copy(wqkv_hbm.at[:, 2 * D:3 * D], wv_v, 6)
    x2_c = x_copy(1024, 2048, 7)
    late = [
        copy(wo_hbm, wo_v, 8),
        copy(w1_hbm, w1_v, 9),
        copy(w2_hbm, w2_v, 10),
        copy(b1_hbm, b1_v, 11),
        copy(b2_hbm, b2_v, 12),
    ]
    for c in [x0a_c, wql_c, x0b_c, wqh_c, wk_c, x1_c, wv_c, x2_c] + late:
        c.start()

    for i in range(NZ):
        z_ref[i] = 0

    def ln_a(r0, n):
        xn = _layernorm(x_v[r0:r0 + n, :].astype(f32)).astype(bf16)
        xn_ref[r0 // 2:(r0 + n) // 2, :] = pltpu.bitcast(xn, u32)

    pend = [[], []]

    def load_xn(r0, n):
        xp = xn_ref[r0 // 2:(r0 + n) // 2, :]
        toks = pend.pop(0)
        pend.append([])
        if toks:
            top = xp[0:8, 0:128]
            for i, tok in enumerate(toks):
                never = jnp.full((8, 128), z_ref[2 + i], jnp.int32) != 0
                top = jnp.where(never, pltpu.bitcast(tok, u32), top)
            xp = jnp.concatenate(
                [jnp.concatenate([top, xp[0:8, 128:]], axis=1), xp[8:]], axis=0)
        return pltpu.bitcast(xp, bf16)

    def store_q(q, r0, n):
        qt = q.astype(bf16).T.astype(f32)
        qt_ref[:, r0:r0 + n] = qt
        for h in range(H):
            par = h % 2
            w0 = h // 2 * 2 * DH
            zero8 = jnp.zeros((8, n), f32)
            row = jax.lax.broadcasted_iota(jnp.int32, (40, n), 0)
            win = jnp.where((row >= par * DH) & (row < (par + 1) * DH), qt[w0:w0 + 40, :], 0.0)
            win = jnp.concatenate([zero8, win], axis=0).astype(bf16)
            qth_ref.at[h][:, r0:r0 + n] = pltpu.bitcast(win, u32)
        za = z_ref[1]
        pend[-1].append(qth_ref[za, 0:8, r0:r0 + 128])
        pend[-1].append(qt_ref[pl.ds(pl.multiple_of(za * 8, 8), 8), r0:r0 + 128])

    def q_part(r0, n, c0, c1):
        return jnp.dot(load_xn(r0, n), wq_v[:, c0:c1], preferred_element_type=f32) * QSCALE

    def mm_k(r0, n):
        return jnp.dot(load_xn(r0, n), wk_v[...], preferred_element_type=f32)

    def store_k(k, r0, n):
        kp = pltpu.bitcast(k.astype(bf16), u32)
        lane = jax.lax.broadcasted_iota(jnp.int32, (n // 2, 128), 1)
        gs = [kp[:, g * 128:(g + 1) * 128] for g in range(NG)]
        ones = jnp.full((n // 2, 128), 0x3F803F80, u32)
        for hp in range(H // 2):
            g, lo = divmod(hp * 2 * DH, 128)
            src = gs[g]
            if lo + 2 * DH > 128:
                src = jnp.where(lane >= 64, gs[g], gs[g + 1])
            if lo != 8:
                src = pltpu.roll(src, (8 - lo) % 128, 1)
            src = jnp.where(lane < 8, ones, src)
            kh_ref[hp, r0 // 2:(r0 + n) // 2, :] = src
            if r0 < NKV:
                nk = min(n, NKV - r0)
                kf_ref[hp, r0:r0 + nk] = pltpu.bitcast(src[0:nk // 2], bf16).astype(f32)
        pend[-1].append(kh_ref[z_ref[1], r0 // 2:r0 // 2 + 8, :])

    def proj_q(r0, n):
        store_q(q_part(r0, n, 0, D), r0, n)

    def proj_k(r0, n):
        store_k(mm_k(r0, n), r0, n)

    def proj_v(r0, n):
        row_n = jax.lax.broadcasted_iota(jnp.int32, (W, n), 0)
        v = jnp.dot(load_xn(r0, n), wv_v[...], preferred_element_type=f32)
        vt = v.astype(bf16).T.astype(f32)
        for h in range(H):
            w0 = (h * DH) // 8 * 8
            off = (h * DH) % 8
            win = vt[w0:w0 + W, :]
            va_ref[h, :, r0:r0 + n] = jnp.where(
                (row_n >= off) & (row_n < off + DH), win, 1.0)
        pend[-1].append(va_ref[z_ref[1], 0:8, r0:r0 + 128])

    row = jax.lax.broadcasted_iota(jnp.int32, (W, TQ), 0)

    class Z:
        def __init__(self):
            self.st = z_ref[0]
            self.ld = z_ref[1]
            self.q = [z_ref[2 + i] for i in range(NP)]
            self.never = [jnp.full((8, 128), z_ref[2 + NP + i], jnp.int32) != 0
                          for i in range(2)]

    def tie(never, tok, x):
        return jnp.where(never, tok, x)

    def max8(s):
        return jnp.max(s.reshape(s.shape[0] // 8, 8, s.shape[1]), axis=0)

    def load_k(h, par, r0, n):
        return pltpu.bitcast(kh_ref[h >> 1, r0 // 2:(r0 + n) // 2, :], bf16)[:, 0:KW[par]]

    def mk_kb(zs, h, par, kb, d, tok=None):
        k = kf_ref[h >> 1, 0:NKV]
        idx8 = jnp.full((8, 128), 8 + par * DH + d, jnp.int32)
        if tok is not None:
            idx8 = tie(zs.never[0], pltpu.bitcast(tok, jnp.int32), idx8)
        idx = jnp.concatenate([idx8] * (NKV // 8), axis=0)
        kb[zs.st, d] = jnp.take_along_axis(k, idx, axis=1)
        return kb[zs.ld, d, 0:8, :]

    def mk_qb(zs, h, par, qb, t, tok=None):
        w0 = (h * DH) // 8 * 8 if isinstance(h, int) else pl.multiple_of((h * DH) // 8 * 8, 8)
        off = 4 * par
        win = qt_ref[pl.ds(w0, W), t * 128:(t + 1) * 128]
        if tok is not None:
            win = jnp.concatenate(
                [tie(zs.never[0], tok, win[g * 8:(g + 1) * 8]) for g in range(W // 8)], axis=0)
        for d in range(DH):
            qb[zs.st, d, :, t * 128:(t + 1) * 128] = jnp.broadcast_to(
                win[off + d:off + d + 1, :], (8, 128))
        return qb[zs.ld, 0, :, t * 128:(t + 1) * 128]

    kbs, qbs, svs, mvs = (kb_a, kb_b), (qb_a, qb_b), (sv_a, sv_b), (mv_a, mv_b)
    mbs, qas = (mb_a, mb_b), (qa_a, qa_b)
    row8 = jax.lax.broadcasted_iota(jnp.int32, (8, TQ), 0)

    def set_qa(zs, h, par, c):
        m = jnp.max(mvs[par][zs.ld, :, c * TQ:(c + 1) * TQ], axis=0, keepdims=True)
        m = jnp.broadcast_to(m.astype(bf16).astype(f32), (8, TQ))
        mbs[c % 2][zs.st] = m
        q = qth_ref[h, :, c * TQ:(c + 1) * TQ]
        neg = jax.lax.shift_right_logical(pltpu.bitcast(-m, u32), jnp.uint32(16))
        top = jnp.where(row8 == 0, neg, q[0:8])
        qas[c % 2][zs.st] = jnp.concatenate([top, q[8:]], axis=0)

    def store_p(zs, r0, p):
        n = p.shape[0]
        a = r0
        while a < r0 + n:
            t = a // R
            b = min(r0 + n, (t + 1) * R)
            p_refs[t].at[zs.st][(a - t * R) // 2:(b - t * R) // 2, :] = pltpu.bitcast(
                p[a - r0:b - r0].astype(bf16), u32)
            a = b

    def stage_qk(zs, h, par, c, j):
        qm = pltpu.bitcast(qas[c % 2][zs.q[j], 0:KW[par] // 2, :], bf16)
        s = jnp.dot(load_k(h, par, STARTS[j], SIZES[j]), qm,
                    preferred_element_type=f32)
        store_p(zs, STARTS[j], jnp.exp2(s))
        return s

    def stage_vexp(zs, par, c, g, zq, tok=None):
        sv = svs[par][zs.ld, g * 16:(g + 1) * 16, c * TQ:(c + 1) * TQ]
        m = mbs[c % 2][zq]
        if tok is not None:
            m = tie(jnp.concatenate([zs.never[0]] * NTL, axis=1),
                    jnp.concatenate([tok] * NTL, axis=1), m)
        store_p(zs, g * 16, jnp.exp2(sv - jnp.concatenate([m, m], axis=0)))

    x0a_c.wait()
    ln_a(0, 256)
    wql_c.wait()
    x0b_c.wait()
    ql0 = q_part(0, 256, 0, 256)
    ln_a(256, 256)
    ql1 = q_part(256, 256, 0, 256)
    wqh_c.wait()
    qs = []
    for r0, ql in ((0, ql0), (256, ql1)):
        for u in range(2):
            qh = q_part(r0 + u * 128, 128, 256, D)
            qs.append(jnp.concatenate([ql[u * 128:(u + 1) * 128], qh], axis=1))
    store_q(qs[0], 0, 128)
    store_q(qs[1], 128, 128)
    wk_c.wait()
    store_q(qs[2], 256, 128)
    store_q(qs[3], 384, 128)
    proj_k(0, 128)
    proj_k(128, 128)
    k2 = mm_k(256, 128)
    k3 = mm_k(384, 128)
    x1_c.wait()
    wv_c.wait()
    store_k(k2, 256, 128)
    store_k(k3, 384, 128)
    ln_a(512, 256)
    proj_v(0, 256)
    ln_a(768, 256)
    proj_v(256, 256)
    proj_q(512, 256)
    q2 = q_part(768, 128, 0, D)
    q3 = q_part(896, 128, 0, D)
    x2_c.wait()
    store_q(q2, 768, 128)
    store_q(q3, 896, 128)
    zs0 = Z()
    h0 = 0
    chk_ref[...] = jnp.zeros(chk_ref.shape, f32)

    def pre_kb(d0, d1):
        for d in range(d0, d1):
            tok = mk_kb(zs0, h0, 0, kb_a, d)
        pend[-1].append(tok)
        for d in range(d0, d1):
            tok = mk_kb(zs0, 1, 1, kb_b, d)
        pend[-1].append(tok)

    def pre_qb(t0, t1):
        for t in range(t0, t1):
            tok = mk_qb(zs0, h0, 0, qb_a, t)
        pend[-1].append(tok)
        for t in list(range(t0, t1)) + list(range(t0 - 8, t1 - 8)):
            tok = mk_qb(zs0, 1, 1, qb_b, t)
        pend[-1].append(tok)

    def pre_sv(c, nk=NKV):
        qm = pltpu.bitcast(qth_ref[h0, 0:KW[0] // 2, c * TQ:(c + 1) * TQ], bf16)
        s = jnp.dot(load_k(h0, 0, 0, nk), qm, preferred_element_type=f32)
        sv_a[zs0.st, 0:nk, c * TQ:(c + 1) * TQ] = s
        mv_a[zs0.st, :, c * TQ:(c + 1) * TQ] = max8(s)

    ln_a(1024, 256)
    proj_k(512, 256)
    ln_a(1280, 256)
    proj_v(512, 256)
    pre_kb(0, 4)
    proj_q(1024, 256)
    ln_a(1536, 256)
    proj_k(768, 256)
    proj_v(768, 256)
    pre_kb(4, 8)
    pre_qb(8, 10)
    proj_q(1280, 256)
    ln_a(1792, 256)
    proj_k(1024, 256)
    proj_v(1024, 256)
    pre_kb(8, 12)
    pre_qb(10, 12)
    proj_q(1536, 256)
    proj_k(1792, 256)
    proj_v(1280, 256)
    pre_kb(12, 16)
    pre_qb(12, 14)
    proj_q(1792, 256)
    proj_k(1280, 256)
    pre_kb(16, 20)
    proj_v(1536, 256)
    pre_qb(14, 16)
    proj_k(1536, 256)
    pre_sv(0)
    proj_v(1792, 256)
    set_qa(zs0, h0, 0, 0)
    for g in range(NKV // 16):
        stage_vexp(zs0, 0, 0, g, zs0.ld)
    pre_sv(1)
    pre_sv(2, NKV // 2)
    pre_sv(3, NKV // 2)
    for n in range(LEAD):
        stage_qk(zs0, h0, 0, 0, n)

    def normalize(zs, h, par, c, acc):
        w0 = pl.multiple_of((h * DH) // 8 * 8, 8)
        off = 4 * par
        l = acc[0:1, :] if par else acc[W - 1:W, :]
        ok = (jnp.abs(acc) < SAFE_ACC) & (l < SAFE_L) & (l > 1.0 / SAFE_L)
        chk_ref[...] = jnp.maximum(chk_ref[...], max8(jnp.where(ok, 0.0, 1.0)))
        o = acc * pl.reciprocal(l, approx=False)
        pltpu.store(ot_ref.at[pl.ds(w0, W), c * TQ:(c + 1) * TQ], o,
                    mask=(row >= off) & (row < off + DH))

    def head(zs, h, par, last=False, filler=None, build=True):
        vacc = None
        extra = {}
        extra2 = {}
        ng = NKV // 16
        j0 = -(-NKV // R) + 1
        for n in range(NT):
            dh, na = divmod(n + LEAD, NT)
            ca, ja = divmod(na, NP)
            c, j = divmod(n, NP)
            s = None
            if last:
                filler(n)
            if not (dh and last):
                s = stage_qk(zs, h + dh, (par + dh) % 2, ca, ja)
            dn, cn = divmod(c + 1, NQ)
            if not (dn and last):
                if j == j0 - 1:
                    set_qa(zs, h + dn, (par + dn) % 2, cn)
                if j0 <= j < NP - 1:
                    k0, k1 = (j - j0) * ng // (NP - 1 - j0), (j + 1 - j0) * ng // (NP - 1 - j0)
                    for g in range(k0, k1):
                        i0 = (g - k0) * 48 + 24
                        stage_vexp(zs, (par + dn) % 2, cn, g, zs.q[j], s[i0:i0 + 8, 0:128])
            if not (last and n >= T0):
                vp = par if n < T0 else 1 - par
                sv_w, mv_w, kb_r, qb_r = svs[vp], mvs[vp], kbs[vp], qbs[vp]
                nn = (n - T0) % NT
                us = list(range(nn * NU // NT, (nn + 1) * NU // NT))
                npt = s.shape[0] // 8 * NTL
                for iu, u in enumerate(us):
                    hf, b, d = VUNITS[u]
                    cols = slice(hf * VT * 128, (hf + 1) * VT * 128)
                    ti, tt = divmod(iu * npt // len(us), NTL)
                    kk = tie(zs.never[0], s[ti * 8:(ti + 1) * 8, tt * 128:(tt + 1) * 128],
                             kb_r[zs.ld, d, b * 8:(b + 1) * 8, :])
                    pr = jnp.concatenate([kk] * VT, axis=1) * qb_r[zs.q[b % 4], d, :, cols]
                    vacc = pr if d == 0 else vacc + pr
                    if d == DH - 1:
                        res = vacc
                        sv_w[zs.st, b * 8:(b + 1) * 8, cols] = res
                        if b > 0:
                            res = jnp.maximum(res, mv_w[zs.ld, :, cols])
                        mv_w[zs.st, :, cols] = res
            bn = n - T0 - 2
            if build and bn >= 0:
                if bn % 2 == 0 and bn // 2 < DH:
                    extra[n + 3] = mk_kb(zs, h + 2, par, kbs[par], bn // 2, s[0:8, 0:128])
                if bn % 2 == 1 and bn // 2 < S // 128:
                    extra2[n + 3] = mk_qb(zs, h + 2, par, qbs[par], bn // 2, s[64:72, 0:128])
            v = va_ref[h, :, j * R:(j + 1) * R]
            if n in extra:
                v = jnp.concatenate([tie(zs.never[1], extra[n], v[0:8]), v[8:]], axis=0)
            if n in extra2:
                v = jnp.concatenate(
                    [v[0:8], tie(zs.never[1], extra2[n], v[8:16]), v[16:]], axis=0)
            o = jnp.dot(v, pltpu.bitcast(p_refs[j][zs.ld], bf16), preferred_element_type=f32)
            acc = o if j == 0 else acc_ref[zs.ld] + o
            if j < NP - 1:
                acc_ref[zs.st] = acc
            else:
                normalize(zs, h, par, c, acc)

    def heads_body(i, carry):
        zs = Z()
        for u in range(2):
            head(zs, i * 2 + u, u)
        return carry

    NLOOP = (H - NPEEL) // 2
    jax.lax.fori_loop(0, NLOOP, heads_body, 0)

    for c in late:
        c.wait()

    def out_copy(i):
        return pltpu.make_async_copy(
            out_v.at[pl.ds(i * RB, RB), :], out_hbm.at[0, pl.ds(i * RB, RB), :], sem_o.at[i])

    def get_o(i):
        r0 = pl.multiple_of(i * RB, RB)
        return ot_ref[:, pl.ds(r0, RB)].T.astype(bf16)

    def attn_out(i, o):
        r0 = pl.multiple_of(i * RB, RB)
        r0h = pl.multiple_of(i * (RB // 2), RB // 2)
        hres = x_v[pl.ds(r0, RB), :].astype(f32) + jnp.dot(
            o, wo_v[...], preferred_element_type=f32)
        hres_ref[pl.ds(r0, RB), :] = hres
        hn_ref[pl.ds(r0h, RB // 2), :] = pltpu.bitcast(_layernorm(hres).astype(bf16), u32)

    def ffn1(i):
        r0h = pl.multiple_of(i * (RB // 2), RB // 2)
        hn = pltpu.bitcast(hn_ref[pl.ds(r0h, RB // 2), :], bf16)
        a = jnp.dot(hn, w1_v[...], preferred_element_type=f32) + b1_v[...].astype(f32)[None, :]
        return _gelu(a).astype(bf16)

    def ffn2(i, a):
        r0 = pl.multiple_of(i * RB, RB)
        y = jnp.dot(a, w2_v[...], preferred_element_type=f32) + b2_v[...].astype(f32)[None, :]
        out_v[pl.ds(r0, RB), :] = (hres_ref[pl.ds(r0, RB), :] + y).astype(bf16)
        out_copy(i).start()

    st = {}

    def filler(n):
        k = n - (NT - 14)
        if k == 0:
            st['o'] = get_o(0)
            st['y'] = []
        if k >= 2 and k % 2 == 0 and (k - 2) // 2 < NG:
            g = (k - 2) // 2
            st['y'].append(jnp.dot(st['o'], wo_v[:, g * 128:(g + 1) * 128],
                                   preferred_element_type=f32))
        if k == 11:
            hres = x_v[0:RB, :].astype(f32) + jnp.concatenate(st['y'], axis=1)
            hres_ref[0:RB, :] = hres
            hn_ref[0:RB // 2, :] = pltpu.bitcast(_layernorm(hres).astype(bf16), u32)

    zs = Z()
    for u in range(NPEEL):
        hh = jnp.int32(H - NPEEL + u) + zs.st
        head(zs, hh, u, last=(u == NPEEL - 1), filler=filler, build=False)

    @pl.when(jnp.max(chk_ref[...]) > 0.5)
    def _():
        def exact(i, carry):
            h = i // NQ
            c0 = pl.multiple_of((i % NQ) * TQ, TQ)
            k = pltpu.bitcast(kh_ref[h >> 1], bf16)[:, 0:KW[1]]
            qm = pltpu.bitcast(qth_ref[h, :, pl.ds(c0, TQ)], bf16)
            s = jnp.dot(k, qm, preferred_element_type=f32)
            p = jnp.exp2(s - jnp.max(s, axis=0, keepdims=True))
            acc = jnp.dot(va_ref[h], p.astype(bf16), preferred_element_type=f32)
            w0 = pl.multiple_of((h * DH) // 8 * 8, 8)
            off = (h * DH) % 8
            l = jnp.where(off == 0, acc[W - 1:W, :], acc[0:1, :])
            pltpu.store(ot_ref.at[pl.ds(w0, W), pl.ds(c0, TQ)], acc / l,
                        mask=(row >= off) & (row < off + DH))
            return carry

        jax.lax.fori_loop(0, H * NQ, exact, 0)
        attn_out(0, get_o(0))

    def c_step(i):
        o = get_o(i + 1)
        a = ffn1(i)
        attn_out(i + 1, o)
        ffn2(i, a)

    def phase_c(i, carry):
        c_step(2 * i)
        c_step(2 * i + 1)
        return carry

    jax.lax.fori_loop(0, (NB - 2) // 2, phase_c, 0)
    zc = z_ref[0]
    c_step(NB - 2 + zc)
    ffn2(NB - 1 + zc, ffn1(NB - 1 + zc))
    for i in range(NB):
        out_copy(i).wait()


@jax.jit
def pallas_sequential_preLN__softmax_full_mha__dense_activation_gelu__prompt_kernel(
    A_x: jax.Array,
    A_wqkv: jax.Array,
    A_wo: jax.Array,
    B_x: jax.Array,
    B_w1: jax.Array,
    B_b1: jax.Array,
    B_w2: jax.Array,
    B_b2: jax.Array,
):
    del B_x
    bf16 = jnp.bfloat16
    f32 = jnp.float32
    u32 = jnp.uint32
    any_spec = pl.BlockSpec(memory_space=pl.ANY)
    return pl.pallas_call(
        _kernel,
        out_shape=jax.ShapeDtypeStruct((1, S, D), bf16),
        in_specs=[any_spec] * 7,
        out_specs=any_spec,
        scratch_shapes=[
            pltpu.VMEM((S, D), bf16),
            pltpu.VMEM((D, D), bf16),
            pltpu.VMEM((D, D), bf16),
            pltpu.VMEM((D, D), bf16),
            pltpu.VMEM((D, D), bf16),
            pltpu.VMEM((D, F), bf16),
            pltpu.VMEM((F, D), bf16),
            pltpu.VMEM((S // 2, D), u32),
            pltpu.VMEM((H // 2, S // 2, 128), u32),
            pltpu.VMEM((H, 24, S), u32),
            pltpu.VMEM((D, S), f32),
            pltpu.VMEM((H, W, S), f32),
            pltpu.VMEM((D, S), f32),
            pltpu.VMEM((S, D), f32),
            pltpu.VMEM((S // 2, D), u32),
            pltpu.VMEM((S, D), bf16),
            pltpu.SMEM((NZ,), jnp.int32),
            pltpu.SemaphoreType.DMA((13,)),
            pltpu.SemaphoreType.DMA((NB,)),
            pltpu.VMEM((1, W, TQ), f32),
            pltpu.VMEM((8, TQ), f32),
            pltpu.VMEM((H // 2, -(-NKV // 32) * 32, 128), f32),
        ] + [pltpu.VMEM((1, DH, NKV, 128), f32)] * 2
          + [pltpu.VMEM((1, DH, 8, S), f32)] * 2
          + [pltpu.VMEM((1, NKV, S), f32)] * 2
          + [pltpu.VMEM((1, 8, S), f32)] * 2
          + [pltpu.VMEM((1, 8, TQ), f32)] * 2
          + [pltpu.VMEM((1, 24, TQ), u32)] * 2
          + [pltpu.VMEM((1, R // 2, TQ), u32)] * NP
          + [pltpu.VMEM((F,), bf16), pltpu.VMEM((D,), bf16)],
        compiler_params=pltpu.CompilerParams(vmem_limit_bytes=110 * 1024 * 1024),
    )(A_x, A_wqkv, A_wo, B_w1, B_b1, B_w2, B_b2)
```

```python
import math

import jax
import jax.numpy as jnp
import jax.experimental.pallas as pl
import jax.experimental.pallas.tpu as pltpu

S = 2048
D = 640
F = 1536
H = 32
DH = D // H
NG = D // 128
EPS = 1e-5

TQ = 512
R = 128
NQ = S // TQ
NP = S // R
NT = NQ * NP
NTL = TQ // 128
W = 24
NPEEL = 2

NKV = 224
NKM = S - NKV
VT = 8
VUNITS = [(hf, b, d) for hf in range(16 // VT) for b in range(NKV // 8) for d in range(DH)]
NU = len(VUNITS)
DG = 5
_U16 = NKM // 16
SIZES = [(_U16 // NP + (1 if i < _U16 % NP else 0)) * 16 for i in range(NP)]
STARTS = [NKV + sum(SIZES[:i]) for i in range(NP)]
LEAD = 2
T0 = NT // 4
SAFE_L = 2.0 ** 60
SAFE_ACC = 2.0 ** 120

RB = 256
NB = S // RB

QSCALE = (DH ** -0.5) * math.log2(math.e)
NZ = 24
KW = (32, 48)


def _layernorm(x):
    m = jnp.mean(x, axis=-1, keepdims=True)
    xc = x - m
    v = jnp.mean(xc * xc, axis=-1, keepdims=True)
    return xc * jax.lax.rsqrt(v + EPS)


def _gelu(x):
    c = math.sqrt(2.0 / math.pi)
    return 0.5 * x * (1.0 + jnp.tanh(c * (x + 0.044715 * (x * x * x))))


def _kernel(x_hbm, wqkv_hbm, wo_hbm, w1_hbm, b1_hbm, w2_hbm, b2_hbm, out_hbm,
            x_v, wq_v, wk_v, wv_v, wo_v, w1_v, w2_v,
            xn_ref, kh_ref, qth_ref, qt_ref, va_ref, ot_ref, hres_ref, hn_ref, out_v,
            z_ref, sem_in, sem_o,
            acc_ref, chk_ref, kf_ref, kb_a, kb_b, qb_a, qb_b, sv_a, sv_b, mv_a, mv_b,
            mb_a, mb_b, qa_a, qa_b, *rest):
    p_refs, (b1_v, b2_v) = rest[:NP], rest[NP:]
    f32 = jnp.float32
    bf16 = jnp.bfloat16
    u32 = jnp.uint32

    def copy(src, dst, i):
        return pltpu.make_async_copy(src, dst, sem_in.at[i])

    def x_copy(r0, r1, i):
        return copy(x_hbm.at[0, r0:r1, :], x_v.at[r0:r1, :], i)

    x0a_c = x_copy(0, 256, 0)
    wql_c = copy(wqkv_hbm.at[:, 0:256], wq_v.at[:, 0:256], 1)
    x0b_c = x_copy(256, 512, 2)
    wqh_c = copy(wqkv_hbm.at[:, 256:D], wq_v.at[:, 256:D], 3)
    wk_c = copy(wqkv_hbm.at[:, D:2 * D], wk_v, 4)
    x1_c = x_copy(512, 1024, 5)
    wv_c = copy(wqkv_hbm.at[:, 2 * D:3 * D], wv_v, 6)
    x2_c = x_copy(1024, 2048, 7)
    late = [
        copy(wo_hbm, wo_v, 8),
        copy(w1_hbm, w1_v, 9),
        copy(w2_hbm, w2_v, 10),
        copy(b1_hbm, b1_v, 11),
        copy(b2_hbm, b2_v, 12),
    ]
    for c in [x0a_c, wql_c, x0b_c, wqh_c, wk_c, x1_c, wv_c, x2_c] + late:
        c.start()

    for i in range(NZ):
        z_ref[i] = 0

    def ln_a(r0, n):
        xn = _layernorm(x_v[r0:r0 + n, :].astype(f32)).astype(bf16)
        xn_ref[r0 // 2:(r0 + n) // 2, :] = pltpu.bitcast(xn, u32)

    pend = [[], []]

    def load_xn(r0, n):
        xp = xn_ref[r0 // 2:(r0 + n) // 2, :]
        toks = pend.pop(0)
        pend.append([])
        if toks:
            top = xp[0:8, 0:128]
            for i, tok in enumerate(toks):
                never = jnp.full((8, 128), z_ref[2 + i], jnp.int32) != 0
                top = jnp.where(never, pltpu.bitcast(tok, u32), top)
            xp = jnp.concatenate(
                [jnp.concatenate([top, xp[0:8, 128:]], axis=1), xp[8:]], axis=0)
        return pltpu.bitcast(xp, bf16)

    def store_q(q, r0, n):
        qt = q.astype(bf16).T.astype(f32)
        qt_ref[:, r0:r0 + n] = qt
        for h in range(H):
            par = h % 2
            w0 = h // 2 * 2 * DH
            zero8 = jnp.zeros((8, n), f32)
            row = jax.lax.broadcasted_iota(jnp.int32, (40, n), 0)
            win = jnp.where((row >= par * DH) & (row < (par + 1) * DH), qt[w0:w0 + 40, :], 0.0)
            win = jnp.concatenate([zero8, win], axis=0).astype(bf16)
            qth_ref.at[h][:, r0:r0 + n] = pltpu.bitcast(win, u32)
        za = z_ref[1]
        pend[-1].append(qth_ref[za, 0:8, r0:r0 + 128])
        pend[-1].append(qt_ref[pl.ds(pl.multiple_of(za * 8, 8), 8), r0:r0 + 128])

    def q_part(r0, n, c0, c1):
        return jnp.dot(load_xn(r0, n), wq_v[:, c0:c1], preferred_element_type=f32) * QSCALE

    def mm_k(r0, n):
        return jnp.dot(load_xn(r0, n), wk_v[...], preferred_element_type=f32)

    def store_k(k, r0, n):
        kp = pltpu.bitcast(k.astype(bf16), u32)
        lane = jax.lax.broadcasted_iota(jnp.int32, (n // 2, 128), 1)
        gs = [kp[:, g * 128:(g + 1) * 128] for g in range(NG)]
        ones = jnp.full((n // 2, 128), 0x3F803F80, u32)
        for hp in range(H // 2):
            g, lo = divmod(hp * 2 * DH, 128)
            src = gs[g]
            if lo + 2 * DH > 128:
                src = jnp.where(lane >= 64, gs[g], gs[g + 1])
            if lo != 8:
                src = pltpu.roll(src, (8 - lo) % 128, 1)
            src = jnp.where(lane < 8, ones, src)
            kh_ref[hp, r0 // 2:(r0 + n) // 2, :] = src
            if r0 < NKV:
                nk = min(n, NKV - r0)
                kf_ref[hp, r0:r0 + nk] = pltpu.bitcast(src[0:nk // 2], bf16).astype(f32)
        pend[-1].append(kh_ref[z_ref[1], r0 // 2:r0 // 2 + 8, :])

    def proj_q(r0, n):
        store_q(q_part(r0, n, 0, D), r0, n)

    def proj_k(r0, n):
        store_k(mm_k(r0, n), r0, n)

    def proj_v(r0, n):
        row_n = jax.lax.broadcasted_iota(jnp.int32, (W, n), 0)
        v = jnp.dot(load_xn(r0, n), wv_v[...], preferred_element_type=f32)
        vt = v.astype(bf16).T.astype(f32)
        masks = [(row_n >= off) & (row_n < off + DH) for off in (0, 4)]
        va_ref[:, :, r0:r0 + n] = jnp.stack(
            [jnp.where(masks[h % 2], vt[(h * DH) // 8 * 8:(h * DH) // 8 * 8 + W, :], 1.0)
             for h in range(H)])
        pend[-1].append(va_ref[z_ref[1], 0:8, r0:r0 + 128])

    row = jax.lax.broadcasted_iota(jnp.int32, (W, TQ), 0)

    class Z:
        def __init__(self):
            self.st = z_ref[0]
            self.ld = z_ref[1]
            self.q = [z_ref[2 + i] for i in range(NP)]
            self.never = [jnp.full((8, 128), z_ref[2 + NP + i], jnp.int32) != 0
                          for i in range(2)]

    def tie(never, tok, x):
        return jax.lax.select(never, tok, x)

    def max8(s):
        return jnp.max(s.reshape(s.shape[0] // 8, 8, s.shape[1]), axis=0)

    def load_k(h, par, r0, n):
        return pltpu.bitcast(kh_ref[h >> 1, r0 // 2:(r0 + n) // 2, :], bf16)[:, 0:KW[par]]

    def mk_kb(zs, h, par, kb, d, tok=None):
        k = kf_ref[h >> 1, 0:NKV]
        idx8 = jnp.full((8, 128), 8 + par * DH + d, jnp.int32)
        if tok is not None:
            idx8 = tie(zs.never[0], pltpu.bitcast(tok, jnp.int32), idx8)
        idx = jnp.concatenate([idx8] * (NKV // 8), axis=0)
        kb[zs.st, d] = jnp.take_along_axis(k, idx, axis=1)
        return kb[zs.ld, d, 0:8, :]

    def mk_qb(zs, h, par, qb, t, tok=None):
        w0 = (h * DH) // 8 * 8 if isinstance(h, int) else pl.multiple_of((h * DH) // 8 * 8, 8)
        off = 4 * par
        win = qt_ref[pl.ds(w0, W), t * 128:(t + 1) * 128]
        if tok is not None:
            win = jnp.concatenate(
                [tie(zs.never[0], tok, win[g * 8:(g + 1) * 8]) for g in range(W // 8)], axis=0)
        qb[zs.st, :, :, t * 128:(t + 1) * 128] = jnp.stack(
            [jnp.broadcast_to(win[off + d:off + d + 1, :], (8, 128)) for d in range(DH)])
        return qb[zs.ld, 0, :, t * 128:(t + 1) * 128]

    kbs, qbs, svs, mvs = (kb_a, kb_b), (qb_a, qb_b), (sv_a, sv_b), (mv_a, mv_b)
    mbs, qas = (mb_a, mb_b), (qa_a, qa_b)
    row8 = jax.lax.broadcasted_iota(jnp.int32, (8, TQ), 0)

    def set_qa(zs, h, par, c):
        m = jnp.max(mvs[par][zs.ld, :, c * TQ:(c + 1) * TQ], axis=0, keepdims=True)
        m = jnp.broadcast_to(m.astype(bf16).astype(f32), (8, TQ))
        mbs[c % 2][zs.st] = m
        q = qth_ref[h, :, c * TQ:(c + 1) * TQ]
        neg = jax.lax.shift_right_logical(pltpu.bitcast(-m, u32), jnp.uint32(16))
        top = jnp.where(row8 == 0, neg, q[0:8])
        qas[c % 2][zs.st] = jnp.concatenate([top, q[8:]], axis=0)

    def store_p(zs, r0, p):
        n = p.shape[0]
        a = r0
        while a < r0 + n:
            t = a // R
            b = min(r0 + n, (t + 1) * R)
            p_refs[t].at[zs.st][(a - t * R) // 2:(b - t * R) // 2, :] = pltpu.bitcast(
                p[a - r0:b - r0].astype(bf16), u32)
            a = b

    def stage_qk(zs, h, par, c, j):
        qm = pltpu.bitcast(qas[c % 2][zs.q[j], 0:KW[par] // 2, :], bf16)
        s = jnp.dot(load_k(h, par, STARTS[j], SIZES[j]), qm,
                    preferred_element_type=f32)
        store_p(zs, STARTS[j], jnp.exp2(s))
        return s

    def stage_vexp(zs, par, c, g, zq, tok=None):
        sv = svs[par][zs.ld, g * 16:(g + 1) * 16, c * TQ:(c + 1) * TQ]
        m = mbs[c % 2][zq]
        if tok is not None:
            m = tie(jnp.concatenate([zs.never[0]] * NTL, axis=1),
                    jnp.concatenate([tok] * NTL, axis=1), m)
        store_p(zs, g * 16, jnp.exp2(sv - jnp.concatenate([m, m], axis=0)))

    x0a_c.wait()
    ln_a(0, 256)
    wql_c.wait()
    x0b_c.wait()
    ql0 = q_part(0, 256, 0, 256)
    ln_a(256, 256)
    ql1 = q_part(256, 256, 0, 256)
    wqh_c.wait()
    qs = []
    for r0, ql in ((0, ql0), (256, ql1)):
        for u in range(2):
            qh = q_part(r0 + u * 128, 128, 256, D)
            qs.append(jnp.concatenate([ql[u * 128:(u + 1) * 128], qh], axis=1))
    store_q(qs[0], 0, 128)
    store_q(qs[1], 128, 128)
    wk_c.wait()
    store_q(qs[2], 256, 128)
    store_q(qs[3], 384, 128)
    proj_k(0, 128)
    proj_k(128, 128)
    k2 = mm_k(256, 128)
    k3 = mm_k(384, 128)
    x1_c.wait()
    wv_c.wait()
    store_k(k2, 256, 128)
    store_k(k3, 384, 128)
    ln_a(512, 256)
    proj_v(0, 256)
    ln_a(768, 256)
    proj_v(256, 256)
    proj_q(512, 256)
    q2 = q_part(768, 128, 0, D)
    q3 = q_part(896, 128, 0, D)
    x2_c.wait()
    store_q(q2, 768, 128)
    store_q(q3, 896, 128)
    zs0 = Z()
    h0 = 0
    chk_ref[...] = jnp.zeros(chk_ref.shape, f32)

    def pre_kb(d0, d1):
        for d in range(d0, d1):
            tok = mk_kb(zs0, h0, 0, kb_a, d)
        pend[-1].append(tok)
        for d in range(d0, d1):
            tok = mk_kb(zs0, 1, 1, kb_b, d)
        pend[-1].append(tok)

    def pre_qb(t0, t1):
        for t in range(t0, t1):
            tok = mk_qb(zs0, h0, 0, qb_a, t)
        pend[-1].append(tok)
        for t in list(range(t0, t1)) + list(range(t0 - 8, t1 - 8)):
            tok = mk_qb(zs0, 1, 1, qb_b, t)
        pend[-1].append(tok)

    def pre_sv(c, nk=NKV):
        qm = pltpu.bitcast(qth_ref[h0, 0:KW[0] // 2, c * TQ:(c + 1) * TQ], bf16)
        s = jnp.dot(load_k(h0, 0, 0, nk), qm, preferred_element_type=f32)
        sv_a[zs0.st, 0:nk, c * TQ:(c + 1) * TQ] = s
        mv_a[zs0.st, :, c * TQ:(c + 1) * TQ] = max8(s)

    ln_a(1024, 256)
    proj_k(512, 256)
    ln_a(1280, 256)
    proj_v(512, 256)
    pre_kb(0, 4)
    proj_q(1024, 256)
    ln_a(1536, 256)
    proj_k(768, 256)
    proj_v(768, 256)
    pre_kb(4, 8)
    pre_qb(8, 10)
    proj_q(1280, 256)
    ln_a(1792, 256)
    proj_k(1024, 256)
    proj_v(1024, 256)
    pre_kb(8, 12)
    pre_qb(10, 12)
    proj_q(1536, 256)
    proj_k(1792, 256)
    proj_v(1280, 256)
    pre_kb(12, 16)
    pre_qb(12, 14)
    proj_q(1792, 256)
    proj_k(1280, 256)
    pre_kb(16, 20)
    proj_v(1536, 256)
    pre_qb(14, 16)
    proj_k(1536, 256)
    pre_sv(0)
    proj_v(1792, 256)
    set_qa(zs0, h0, 0, 0)
    for g in range(NKV // 16):
        stage_vexp(zs0, 0, 0, g, zs0.ld)
    pre_sv(1)
    pre_sv(2, NKV // 2)
    pre_sv(3, NKV // 2)
    for n in range(LEAD):
        stage_qk(zs0, h0, 0, 0, n)

    def normalize(zs, h, par, c, acc):
        w0 = pl.multiple_of((h * DH) // 8 * 8, 8)
        off = 4 * par
        l = acc[0:1, :] if par else acc[W - 1:W, :]
        ok = (jnp.abs(acc) < SAFE_ACC) & (l < SAFE_L) & (l > 1.0 / SAFE_L)
        chk_ref[...] = jnp.maximum(chk_ref[...], max8(jnp.where(ok, 0.0, 1.0)))
        o = acc * pl.reciprocal(l, approx=False)
        pltpu.store(ot_ref.at[pl.ds(w0, W), c * TQ:(c + 1) * TQ], o,
                    mask=(row >= off) & (row < off + DH))

    def head(zs, h, par, last=False, filler=None, build=True):
        vacc = None
        extra = {}
        extra2 = {}
        ng = NKV // 16
        j0 = -(-NKV // R) + 1
        for n in range(NT):
            dh, na = divmod(n + LEAD, NT)
            ca, ja = divmod(na, NP)
            c, j = divmod(n, NP)
            s = None
            if last:
                filler(n)
            if not (dh and last):
                s = stage_qk(zs, h + dh, (par + dh) % 2, ca, ja)
            dn, cn = divmod(c + 1, NQ)
            if not (dn and last):
                if j == j0 - 1:
                    set_qa(zs, h + dn, (par + dn) % 2, cn)
                if j0 <= j < NP - 1:
                    k0, k1 = (j - j0) * ng // (NP - 1 - j0), (j + 1 - j0) * ng // (NP - 1 - j0)
                    for g in range(k0, k1):
                        i0 = (g - k0) * 48 + 24
                        stage_vexp(zs, (par + dn) % 2, cn, g, zs.q[j], s[i0:i0 + 8, 0:128])
            if not (last and n >= T0):
                vp = par if n < T0 else 1 - par
                sv_w, mv_w, kb_r, qb_r = svs[vp], mvs[vp], kbs[vp], qbs[vp]
                nn = (n - T0) % NT
                us = list(range(nn * NU // NT, (nn + 1) * NU // NT))
                npt = s.shape[0] // 8 * NTL
                for iu, u in enumerate(us):
                    hf, b, d = VUNITS[u]
                    cols = slice(hf * VT * 128, (hf + 1) * VT * 128)
                    ti, tt = divmod(iu * npt // len(us), NTL)
                    if d % DG == 0:
                        kg = kb_r[zs.ld, d:d + DG, b * 8:(b + 1) * 8, :]
                        qg = qb_r[zs.q[b % 4], d:d + DG, :, cols]
                    kk = tie(zs.never[0], s[ti * 8:(ti + 1) * 8, tt * 128:(tt + 1) * 128],
                             kg[d % DG])
                    pr = jnp.concatenate([kk] * VT, axis=1) * qg[d % DG]
                    vacc = pr if d == 0 else vacc + pr
                    if d == DH - 1:
                        res = vacc
                        sv_w[zs.st, b * 8:(b + 1) * 8, cols] = res
                        if b > 0:
                            res = jnp.maximum(res, mv_w[zs.ld, :, cols])
                        mv_w[zs.st, :, cols] = res
            bn = n - T0 - 2
            if build and bn >= 0:
                if bn % 2 == 0 and bn // 2 < DH:
                    extra[n + 3] = mk_kb(zs, h + 2, par, kbs[par], bn // 2, s[0:8, 0:128])
                if bn % 2 == 1 and bn // 2 < S // 128:
                    extra2[n + 3] = mk_qb(zs, h + 2, par, qbs[par], bn // 2, s[64:72, 0:128])
            v = va_ref[h, :, j * R:(j + 1) * R]
            if n in extra:
                v = jnp.concatenate([tie(zs.never[1], extra[n], v[0:8]), v[8:]], axis=0)
            if n in extra2:
                v = jnp.concatenate(
                    [v[0:8], tie(zs.never[1], extra2[n], v[8:16]), v[16:]], axis=0)
            o = jnp.dot(v, pltpu.bitcast(p_refs[j][zs.ld], bf16), preferred_element_type=f32)
            acc = o if j == 0 else acc_ref[zs.ld] + o
            if j < NP - 1:
                acc_ref[zs.st] = acc
            else:
                normalize(zs, h, par, c, acc)

    def heads_body(i, carry):
        zs = Z()
        for u in range(2):
            head(zs, i * 2 + u, u)
        return carry

    NLOOP = (H - NPEEL) // 2
    jax.lax.fori_loop(0, NLOOP, heads_body, 0)

    for c in late:
        c.wait()

    def out_copy(i):
        return pltpu.make_async_copy(
            out_v.at[pl.ds(i * RB, RB), :], out_hbm.at[0, pl.ds(i * RB, RB), :], sem_o.at[i])

    def get_o(i):
        r0 = pl.multiple_of(i * RB, RB)
        return ot_ref[:, pl.ds(r0, RB)].T.astype(bf16)

    def attn_out(i, o):
        r0 = pl.multiple_of(i * RB, RB)
        r0h = pl.multiple_of(i * (RB // 2), RB // 2)
        hres = x_v[pl.ds(r0, RB), :].astype(f32) + jnp.dot(
            o, wo_v[...], preferred_element_type=f32)
        hres_ref[pl.ds(r0, RB), :] = hres
        hn_ref[pl.ds(r0h, RB // 2), :] = pltpu.bitcast(_layernorm(hres).astype(bf16), u32)

    def ffn1(i):
        r0h = pl.multiple_of(i * (RB // 2), RB // 2)
        hn = pltpu.bitcast(hn_ref[pl.ds(r0h, RB // 2), :], bf16)
        a = jnp.dot(hn, w1_v[...], preferred_element_type=f32) + b1_v[...].astype(f32)[None, :]
        return _gelu(a).astype(bf16)

    def ffn2(i, a):
        r0 = pl.multiple_of(i * RB, RB)
        y = jnp.dot(a, w2_v[...], preferred_element_type=f32) + b2_v[...].astype(f32)[None, :]
        out_v[pl.ds(r0, RB), :] = (hres_ref[pl.ds(r0, RB), :] + y).astype(bf16)
        out_copy(i).start()

    st = {}

    def filler(n):
        k = n - (NT - 22)
        if k == 0:
            st['o'] = get_o(0)
            st['y'] = []
        if k >= 2 and k % 2 == 0 and (k - 2) // 2 < NG:
            g = (k - 2) // 2
            st['y'].append(jnp.dot(st['o'], wo_v[:, g * 128:(g + 1) * 128],
                                   preferred_element_type=f32))
        if k == 11:
            hres = x_v[0:RB, :].astype(f32) + jnp.concatenate(st['y'], axis=1)
            hres_ref[0:RB, :] = hres
            hn_ref[0:RB // 2, :] = pltpu.bitcast(_layernorm(hres).astype(bf16), u32)

    zs = Z()
    for u in range(NPEEL):
        hh = jnp.int32(H - NPEEL + u) + zs.st
        head(zs, hh, u, last=(u == NPEEL - 1), filler=filler, build=False)

    @pl.when(jnp.max(chk_ref[...]) > 0.5)
    def _():
        def exact(i, carry):
            h = i // NQ
            c0 = pl.multiple_of((i % NQ) * TQ, TQ)
            k = pltpu.bitcast(kh_ref[h >> 1], bf16)[:, 0:KW[1]]
            qm = pltpu.bitcast(qth_ref[h, :, pl.ds(c0, TQ)], bf16)
            s = jnp.dot(k, qm, preferred_element_type=f32)
            p = jnp.exp2(s - jnp.max(s, axis=0, keepdims=True))
            acc = jnp.dot(va_ref[h], p.astype(bf16), preferred_element_type=f32)
            w0 = pl.multiple_of((h * DH) // 8 * 8, 8)
            off = (h * DH) % 8
            l = jnp.where(off == 0, acc[W - 1:W, :], acc[0:1, :])
            pltpu.store(ot_ref.at[pl.ds(w0, W), pl.ds(c0, TQ)], acc / l,
                        mask=(row >= off) & (row < off + DH))
            return carry

        jax.lax.fori_loop(0, H * NQ, exact, 0)
        attn_out(0, get_o(0))

    def c_step(i):
        o = get_o(i + 1)
        a = ffn1(i)
        attn_out(i + 1, o)
        ffn2(i, a)

    def phase_c(i, carry):
        c_step(2 * i)
        c_step(2 * i + 1)
        return carry

    jax.lax.fori_loop(0, (NB - 2) // 2, phase_c, 0)
    zc = z_ref[0]
    c_step(NB - 2 + zc)
    ffn2(NB - 1 + zc, ffn1(NB - 1 + zc))
    for i in range(NB):
        out_copy(i).wait()


@jax.jit
def pallas_sequential_preLN__softmax_full_mha__dense_activation_gelu__prompt_kernel(
    A_x: jax.Array,
    A_wqkv: jax.Array,
    A_wo: jax.Array,
    B_x: jax.Array,
    B_w1: jax.Array,
    B_b1: jax.Array,
    B_w2: jax.Array,
    B_b2: jax.Array,
):
    del B_x
    bf16 = jnp.bfloat16
    f32 = jnp.float32
    u32 = jnp.uint32
    any_spec = pl.BlockSpec(memory_space=pl.ANY)
    return pl.pallas_call(
        _kernel,
        out_shape=jax.ShapeDtypeStruct((1, S, D), bf16),
        in_specs=[any_spec] * 7,
        out_specs=any_spec,
        scratch_shapes=[
            pltpu.VMEM((S, D), bf16),
            pltpu.VMEM((D, D), bf16),
            pltpu.VMEM((D, D), bf16),
            pltpu.VMEM((D, D), bf16),
            pltpu.VMEM((D, D), bf16),
            pltpu.VMEM((D, F), bf16),
            pltpu.VMEM((F, D), bf16),
            pltpu.VMEM((S // 2, D), u32),
            pltpu.VMEM((H // 2, S // 2, 128), u32),
            pltpu.VMEM((H, 24, S), u32),
            pltpu.VMEM((D, S), f32),
            pltpu.VMEM((H, W, S), f32),
            pltpu.VMEM((D, S), f32),
            pltpu.VMEM((S, D), f32),
            pltpu.VMEM((S // 2, D), u32),
            pltpu.VMEM((S, D), bf16),
            pltpu.SMEM((NZ,), jnp.int32),
            pltpu.SemaphoreType.DMA((13,)),
            pltpu.SemaphoreType.DMA((NB,)),
            pltpu.VMEM((1, W, TQ), f32),
            pltpu.VMEM((8, TQ), f32),
            pltpu.VMEM((H // 2, -(-NKV // 32) * 32, 128), f32),
        ] + [pltpu.VMEM((1, DH, NKV, 128), f32)] * 2
          + [pltpu.VMEM((1, DH, 8, S), f32)] * 2
          + [pltpu.VMEM((1, NKV, S), f32)] * 2
          + [pltpu.VMEM((1, 8, S), f32)] * 2
          + [pltpu.VMEM((1, 8, TQ), f32)] * 2
          + [pltpu.VMEM((1, 24, TQ), u32)] * 2
          + [pltpu.VMEM((1, R // 2, TQ), u32)] * NP
          + [pltpu.VMEM((F,), bf16), pltpu.VMEM((D,), bf16)],
        compiler_params=pltpu.CompilerParams(vmem_limit_bytes=110 * 1024 * 1024),
    )(A_x, A_wqkv, A_wo, B_w1, B_b1, B_w2, B_b2)
```
